```python
import jax
import jax.numpy as jnp

def _softmax(x, axis=-1):
    return jax.nn.softmax(x, axis=axis)
def _gelu(x):
    return jax.nn.gelu(x, approximate=True)
def _silu(x):
    return jax.nn.silu(x)
def _sigmoid(x):
    return jax.nn.sigmoid(x)
def _layernorm(x, axis=-1, eps=1e-5):
    m = jnp.mean(x, axis=axis, keepdims=True)
    v = jnp.var(x, axis=axis, keepdims=True)
    return (x - m) / jnp.sqrt(v + eps)
def _scatter_add(tgt, idx, src, axis=0):
    return tgt.at[idx].add(src)
def _segment_sum(src, seg, n):
    return jax.ops.segment_sum(src, seg, n)
class _Rng:
    def __init__(self, key):
        self._k = key
    def _next(self):
        self._k, sub = jax.random.split(self._k)
        return sub
    def normal(self, shape):
        return jax.random.normal(self._next(), shape, dtype=jnp.bfloat16)
    def randint(self, lo, hi, shape):
        return jax.random.randint(self._next(), shape, lo, hi, dtype=jnp.int32)
    def uniform(self, shape, lo=0.0, hi=1.0):
        return jax.random.uniform(self._next(), shape, jnp.bfloat16, lo, hi)
    def permutation(self, n):
        return jax.random.permutation(self._next(), n)


kernel_name = 'recurrent_scan__compressed_kv_cla__dense_activation_gelu__decode'

def setup_inputs():
    _rng = _Rng(jax.random.key(int.from_bytes(__import__("os").urandom(4), "little")))
    _w = (lambda a: (lambda t: t.astype(jnp.bfloat16) if jnp.issubdtype(t.dtype, jnp.floating) else t)(jnp.asarray(a)))
    def _A_setup():
        B, H, Sq, Sk, D, M = 2, 32, 1, 16384, 128, 512
        Dc = 4 * D
        return {
            "x": _w((lambda *s: _rng.normal(s) * 0.05)(B, Sq, M)),
            "c_kv": _w((lambda *s: _rng.normal(s) * 0.05)(B, Sk, Dc)),
            "w_q": _w((lambda *s: _rng.normal(s) * 0.05)(M, H, D) * (M ** -0.5)),
            "w_uk": _w((lambda *s: _rng.normal(s) * 0.05)(Dc, H, D) * (Dc ** -0.5)),
            "w_uv": _w((lambda *s: _rng.normal(s) * 0.05)(Dc, H, D) * (Dc ** -0.5)),
            "w_o": _w((lambda *s: _rng.normal(s) * 0.05)(H, D, M) * ((H * D) ** -0.5)),
        }
    _A_in = _A_setup()

    def _B_setup():
        B, S, D, F = 2, 1, 512, 1792
        return {
            "x": _w((lambda *s: _rng.normal(s) * 0.05)(B, S, D)),
            "w1": _w((lambda *s: _rng.normal(s) * 0.05)(D, F) * (D ** -0.5)),
            "b1": _w((lambda *s: _rng.normal(s) * 0.05)(F) * 0.01),
            "w2": _w((lambda *s: _rng.normal(s) * 0.05)(F, D) * (F ** -0.5)),
            "b2": _w((lambda *s: _rng.normal(s) * 0.05)(D) * 0.01),
        }
    _B_in = _B_setup()

    return {
        "A_x": _A_in["x"],
        "A_c_kv": _A_in["c_kv"],
        "A_w_q": _A_in["w_q"],
        "A_w_uk": _A_in["w_uk"],
        "A_w_uv": _A_in["w_uv"],
        "A_w_o": _A_in["w_o"],
        "B_x": _B_in["x"],
        "B_w1": _B_in["w1"],
        "B_b1": _B_in["b1"],
        "B_w2": _B_in["w2"],
        "B_b2": _B_in["b2"],
    }

def reference(A_x, A_c_kv, A_w_q, A_w_uk, A_w_uv, A_w_o, B_x, B_w1, B_b1, B_w2, B_b2):
    def _A_ref(x, c_kv, w_q, w_uk, w_uv, w_o):
        B, Sq, M = x.shape[0], x.shape[1], x.shape[2]
        Sk = c_kv.shape[1]
        H, D = w_q.shape[1], w_q.shape[2]
        q = jnp.einsum("bqm,mhd->bhqd", x, w_q)
        k = jnp.einsum("bkc,chd->bhkd", c_kv, w_uk)
        v = jnp.einsum("bkc,chd->bhkd", c_kv, w_uv)
        scores = jnp.einsum("bhqd,bhkd->bhqk", q, k) * (D ** -0.5)
        off = Sk - Sq
        qi = jnp.arange(Sq)[:, None]
        kj = jnp.arange(Sk)[None, :]
        cmask = kj <= (qi + off)
        scores = jnp.where(cmask[None, None], scores, -1e9)
        p = _softmax(scores, axis=-1)
        ctx = jnp.einsum("bhqk,bhkd->bhqd", p, v)
        return jnp.einsum("bhqd,hdm->bqm", ctx, w_o)

    def _B_ref(x, w1, b1, w2, b2):
        h = jnp.einsum("bsd,df->bsf", x, w1) + b1
        h = _gelu(h)
        return jnp.einsum("bsf,fd->bsd", h, w2) + b2

    x = A_x
    xn = _layernorm(x, axis=-1)
    s = _A_ref(xn, A_c_kv, A_w_q, A_w_uk, A_w_uv, A_w_o)
    g = _silu(_B_ref(xn, B_w1, B_b1, B_w2, B_b2))
    return x + s * g
```

```python
import contextlib
import jax
import jax.numpy as jnp
from jax import lax
import jax.experimental.pallas as pl
import jax.experimental.pallas.tpu as pltpu

F32 = jnp.float32
BF16 = jnp.bfloat16

B, H, SK, D, M, DC, F = 2, 32, 16384, 128, 512, 512, 1792
LOG2E = 1.4426950408889634
NT = (((1,), (1,)), ((), ()))

C_VIEW = (2048, 16, DC)
W_VIEW = (256, 2 * H, D)
O_VIEW = (256, 16, M)
W1_VIEW = (112, 64, 128)
W2_VIEW = (112, 16, M)
NBLK = 32


def _loop(lo, hi, body):
    lax.fori_loop(lo, hi, lambda i, _: body(i), None)


def _rows8(v):
    return jnp.concatenate([v[:, j * 128:(j + 1) * 128] for j in range(M // 128)], axis=0)


def natural(runs, k=None):
    k = k or len(runs)
    return [r * 4 + t for g in range(0, len(runs), k) for t in range(4) for r in runs[g:g + k]]


EVEN_ODD = [0, 2, 4, 6, 8, 10, 12, 14, 1, 3, 5, 7, 9, 11, 13, 15]
MXU_HEADS = ([4 * r + k for k in (0, 1) for r in range(8)], [4 * r + 2 for r in range(8)], [3, 11, 19, 27])
VPU_HEADS = [7, 15, 23, 31]


def order_o():
    out = []
    for heads in MXU_HEADS + (VPU_HEADS,):
        for g in range(0, len(heads), 8):
            hs = heads[g:g + 8]
            hs = hs[0::2] + hs[1::2] if len(hs) == 8 else hs
            out += [h * 8 + t for t in range(8) for h in hs]
    return out


def make(QA=None, QB=None, QC=None, QD=None, skew=(2, 2, 2, 2, 2, 3), lag=8, small=8, nsmall=4,
         cuts=(12, 20, 26, 30, 31, 32), dcut=(32, 42, 46, 50, 54), dma_only=False, TR=False, mxu_heads=MXU_HEADS, vpu_heads=VPU_HEADS):
    QA = QA or natural(EVEN_ODD)
    QB = QB or natural([0, 2, 4, 6, 8, 10, 11, 13, 1, 3, 5, 7, 9, 12, 14])
    QC = QC or natural(list(range(16)))
    QD = QD or order_o()
    assert sorted(QA) == sorted(QC) == list(range(64)) and sorted(QB) == list(range(60)) and sorted(QD) == list(range(256))
    NV = len(vpu_heads) * 8
    assert sorted(QD[-NV:]) == sorted(h * 8 + t for h in vpu_heads for t in range(8)) and cuts[-1] == NV
    s_c, s_q, s_k, s_v, s_1, s_2 = skew
    scope = (lambda n: jax.named_scope('@' + n)) if TR else (lambda n: contextlib.nullcontext())

    def kernel(x_hbm, ckv_hbm, wq_hbm, wuk_hbm, wuv_hbm, wo_hbm, w1_hbm, b1_hbm, w2_hbm, b2_hbm,
               o_hbm,
               x_buf, b1_buf, b2_buf, c_buf, wq_buf, wuk_buf, wuv_buf, wo_buf, w1_buf, w2_buf,
               qa_ref, acc_ref, m_ref, l_ref, a_buf, e_buf, ctx_ref, mul_ref, o_buf,
               sem_w, sem_c, sem_o, sem_last, sem_small):
        def piece(hbm, buf, i, sem):
            return pltpu.make_async_copy(hbm.at[i], buf.at[i], sem)

        def wait_filled(buf, sem):
            pltpu.make_async_copy(buf, buf, sem).wait()

        def wrap(j, last, off, n):
            i = 4 * j + off
            if 4 * last + off < n:
                return i
            return i % n if isinstance(i, int) else jnp.where(i >= n, i - n, i)

        def round_a(j):
            def one(e):
                r, t = divmod(e, 4)
                hbm, buf, s = (wq_hbm, wq_buf, s_q) if r >= 8 else (wuk_hbm, wuk_buf, s_k)
                return piece(hbm, buf, wrap(j, 7, s + (r % 8) * 32 + t, 256), sem_w.at[0])
            return [lambda e=e: one(e) for e in QA]

        def round_b(j, half):
            def one(e):
                r, t = divmod(e, 4)
                if r < 8:
                    return piece(wuv_hbm, wuv_buf, wrap(j, 7, s_v + r * 32 + t, 256), sem_w.at[1])
                if r == 14:
                    hbm, buf, s = (w2_hbm, w2_buf, s_2) if half else (w1_hbm, w1_buf, s_1)
                    return piece(hbm, buf, wrap(j, 3 + 4 * half, s + 96 - 16 * half + t, 112), sem_w.at[1])
                hbm, buf, s = (w2_hbm, w2_buf, s_2) if r >= 11 else (w1_hbm, w1_buf, s_1)
                return piece(hbm, buf, 4 * j + (s + ((r - 8) % 3) * 32 + t), sem_w.at[1])
            return [lambda e=e: one(e) for e in QB]

        def round_c(i):
            j, b = i >> 1, i & 1

            def one(e):
                r, t = divmod(e, 4)
                return pltpu.make_async_copy(ckv_hbm.at[b * 1024 + wrap(j, 15, s_c + r * 64 + t, 1024)],
                                             c_buf.at[i, e], sem_c.at[i])
            return [lambda e=e: one(e) for e in QC]

        def sem_d(n):
            if n >= 256 - NV:
                return sem_last.at[sum(n - (256 - NV) >= c for c in cuts)]
            return sem_o.at[[QD[n] // 8 in hs for hs in mxu_heads].index(True)]

        big = 256 - small
        stream_d = [lambda n=n: piece(wo_hbm, wo_buf, QD[n], sem_d(n)) for n in range(big)]

        def issue(cur, nxt, lo, hi):
            seq = cur + nxt
            for g in range(lo, min(hi, len(cur) // 4)):
                if g >= 0:
                    seq[4 * g]().start(priority=0)
                for c in seq[4 * (g + lag) + 1:4 * (g + lag) + 4]:
                    c().start(priority=1)

        def issue_end(lo, hi):
            parts = []
            for n in range(big, 256):
                w = 16 * M // 8 // nsmall
                for u in range(nsmall):
                    ix = (QD[n], pl.ds(u * w // M * 8, 8), pl.ds(u * w % M, w))
                    parts.append(lambda n=n, ix=ix: pltpu.make_async_copy(wo_hbm.at[ix], wo_buf.at[ix], sem_d(n)))
            pad = []
            for g in range(0, len(parts), 3):
                pad += [None] + parts[g:g + 3]
            issue(stream_d, pad, lo, hi)
            if hi >= big // 4:
                for c in parts[3 * lag:]:
                    c().start(priority=1)

        x_copy = pltpu.make_async_copy(x_hbm, x_buf, sem_small.at[0])
        b1_copy = pltpu.make_async_copy(b1_hbm, b1_buf, sem_small.at[1])
        b2_copy = pltpu.make_async_copy(b2_hbm, b2_buf, sem_small.at[2])

        first = round_a(0)
        first[0]().start(priority=0)
        issue(first, [], -lag, 0)
        for c in first[4 * lag + 1:4 * lag + 4]:
            c().start(priority=1)
        issue(first, round_a(1), 1, 16)
        for c in (x_copy, b1_copy, b2_copy):
            c.start()
        _loop(1, 4, lambda j: issue(round_a(j), round_a(j + 1), 0, 16))

        if dma_only:
            _loop(4, 7, lambda j: issue(round_a(j), round_a(j + 1), 0, 16))
            issue(round_a(7), round_b(0, 0), 0, 16)
            _loop(0, 3, lambda j: issue(round_b(j, 0), round_b(j + 1, 0), 0, 16))
            issue(round_b(3, 0), round_b(4, 1), 0, 16)
            _loop(4, 7, lambda j: issue(round_b(j, 1), round_b(j + 1, 1), 0, 16))
            issue(round_b(7, 1), round_c(0), 0, 16)
            _loop(0, 31, lambda i: issue(round_c(i), round_c(i + 1), 0, 16))
            issue(round_c(31), stream_d, 0, 16)
            issue_end(0, 64)
            for c in (x_copy, b1_copy, b2_copy):
                c.wait()
            for v in (wq_buf, wuk_buf):
                wait_filled(v, sem_w.at[0])
            for v in (wuv_buf, w1_buf, w2_buf):
                wait_filled(v, sem_w.at[1])
            for i in range(NBLK):
                wait_filled(c_buf.at[i], sem_c.at[i])
            for g, hs in enumerate(mxu_heads):
                wait_filled(wo_buf.at[pl.ds(0, 8 * len(hs))], sem_o.at[g])
            for i, (lo, hi) in enumerate(zip((0,) + cuts, cuts)):
                wait_filled(wo_buf.at[pl.ds(0, hi - lo)], sem_last.at[i])
            o_copy = pltpu.make_async_copy(o_buf, o_hbm, sem_small.at[0])
            o_copy.start()
            o_copy.wait()
            return

        with scope('x'):
            x_copy.wait()
        x = x_buf[...].astype(F32)
        xc = x - jnp.mean(x, axis=-1, keepdims=True)
        var = jnp.mean(xc * xc, axis=-1, keepdims=True)
        xn = (xc * lax.rsqrt(var + 1e-5)).astype(BF16)
        e_buf[...] = (lax.broadcasted_iota(jnp.int32, (128, 1024), 1) // 8
                      == lax.broadcasted_iota(jnp.int32, (128, 1024), 0)).astype(F32).astype(BF16)
        m_ref[...] = jnp.full((B * H, 128), -jnp.inf, F32)
        l_ref[...] = jnp.zeros((B * H, 128), F32)
        acc_ref[...] = jnp.zeros((B * H, DC), F32)

        def own_head(v):
            keep = (lax.broadcasted_iota(jnp.int32, v.shape, 0) % 8 == lax.broadcasted_iota(jnp.int32, v.shape, 1) % 8)
            return jnp.where(keep, v, 0.0).astype(BF16)

        def spread(v):
            return own_head(jnp.dot(v, e_buf[...], preferred_element_type=F32))

        def heads(buf, j):
            w = buf[pl.ds(j * 64, 64)].reshape(128, 4, 8, D)
            return [w[:, g].reshape(1024, D) for g in range(4)]

        xf = xn.astype(F32)
        x16 = jnp.concatenate([jnp.broadcast_to(xf[b:b + 1], (8, M)) for b in range(B)], axis=0).astype(BF16)
        for j in range(4):
            a_buf[j, :16] = spread(x16[:, j * 128:(j + 1) * 128])
        with scope('a4'):
            _loop(4, 7, lambda j: issue(round_a(j), round_a(j + 1), 0, 16))
            issue(round_a(7), round_b(0, 0), 0, 16)

        def q_round(j, q):
            with scope('b0'):
                issue(round_b(j, 0), round_b(j + 1, 0), 0, 16)

            @pl.when(j == 1)
            def _():
                with scope('wq'):
                    wait_filled(wq_buf, sem_w.at[0])
                    wait_filled(wuk_buf, sem_w.at[0])

            def part(i, q):
                return tuple(t + jnp.dot(a_buf[i, :16], w, preferred_element_type=F32) for t, w in zip(q, heads(wq_buf, i)))
            return lax.fori_loop(jnp.maximum(2 * j - 2, 0), 2 * j, part, q)

        q = lax.fori_loop(0, 3, q_round, (jnp.zeros((16, D), F32),) * 4)
        q = [t.astype(BF16) for t in q]

        def qa_round(j):
            with scope('b3'):
                pl.when(j == 3)(lambda: issue(round_b(3, 0), round_b(4, 1), 0, 16))
                pl.when(j > 3)(lambda: issue(round_b(j, 1), round_b(j + 1, 1), 0, 16))
            r = [lax.dot_general(t, w, NT, preferred_element_type=F32) for t, w in zip(q, heads(wuk_buf, j - 3))]
            r = jnp.concatenate([t[8 * b:8 * b + 8] for b in range(B) for t in r], axis=0)
            r = own_head(r * (D ** -0.5 * LOG2E))
            qa_ref[j - 3] = lax.dot_general(r, e_buf[...], NT, preferred_element_type=F32).astype(BF16)

        _loop(3, 7, qa_round)
        with scope('b7'):
            issue(round_b(7, 1), round_c(0), 0, 16)
            _loop(0, 2, lambda i: issue(round_c(i), round_c(i + 1), 0, 16))

        with scope('w1'):
            for v in (wuv_buf, w1_buf, w2_buf):
                wait_filled(v, sem_w.at[1])
            b1_copy.wait()
            b2_copy.wait()
        w1 = w1_buf[...].reshape(M // 8, F // 128, 8, 128)
        hid = jnp.concatenate([jnp.dot(xn, w1[:, j].reshape(M, 128), preferred_element_type=F32)
                               for j in range(F // 128)], axis=1)
        hid = jax.nn.gelu(hid + b1_buf[...].astype(F32).reshape(1, F), approximate=True).astype(BF16)
        z = jnp.dot(hid, w2_buf[...].reshape(F, M), preferred_element_type=F32)
        z8 = _rows8(z + b2_buf[...].astype(F32).reshape(1, M))
        g8 = z8 * jax.nn.sigmoid(z8)
        x8 = _rows8(x)

        def feed(i, half):
            lo, hi = 8 * half, 8 * half + 8
            with scope('c'):
                pl.when(i < NBLK - 1)(lambda: issue(round_c(i), round_c(i + 1), lo, hi))
                pl.when(i == NBLK - 1)(lambda: issue(round_c(NBLK - 1), stream_d, lo, hi))
                pl.when(i == NBLK)(lambda: issue_end(lo, hi))
                pl.when(i == NBLK + 1)(lambda: issue_end(16 + lo, 16 + hi))

        def block(i):
            feed(i + 2, 0)
            with scope('wc'):
                wait_filled(c_buf.at[i], sem_c.at[i])
            hrows = pl.ds(pl.multiple_of((i & 1) * H, H), H)
            qa = jnp.concatenate([qa_ref[j, hrows] for j in range(4)], axis=1)
            sc = lax.dot_general(qa, c_buf[i].reshape(1024, DC), NT, preferred_element_type=F32)
            m_prev = m_ref[hrows, :]
            m_new = jnp.maximum(m_prev, jnp.max(sc, axis=1, keepdims=True))
            p = [jnp.exp2(sc[:, j * 128:(j + 1) * 128] - m_new) for j in range(8)]
            alpha = jnp.exp2(m_prev - m_new)
            l_ref[hrows, :] = alpha * l_ref[hrows, :] + sum(p)
            m_ref[hrows, :] = m_new
            p = jnp.concatenate(p, axis=1).astype(BF16)
            feed(i + 2, 1)
            pv = jnp.dot(p, c_buf[i].reshape(1024, DC), preferred_element_type=F32)
            acc_ref[hrows, :] = acc_ref[hrows, :] * jnp.concatenate([alpha] * 4, axis=1) + pv

        _loop(0, NBLK, block)

        pc = acc_ref[...] / jnp.sum(l_ref[...], axis=1, keepdims=True)
        pc = jnp.concatenate([pc[b * H + 8 * g:b * H + 8 * g + 8] for g in range(4) for b in range(B)], axis=0).astype(BF16)
        a = spread(jnp.concatenate([pc[:, j * 128:(j + 1) * 128] for j in range(4)], axis=0))
        a_buf[...] = a.reshape(4, B * H, 1024)

        def ctx_part(j, ctx):
            with scope('d'):
                for k, (lo, hi) in enumerate(zip(dcut[:4], dcut[1:])):
                    pl.when(j == k)(lambda: issue_end(lo, hi))
            return tuple(t + jnp.dot(a_buf[j, 16 * g:16 * g + 16], w, preferred_element_type=F32)
                         for g, (t, w) in enumerate(zip(ctx, heads(wuv_buf, j))))

        ctx = lax.fori_loop(0, 4, ctx_part, (jnp.zeros((16, D), F32),) * 4)
        ctx = jnp.concatenate([t[8 * b:8 * b + 8] for b in range(B) for t in ctx], axis=0)
        ctx_ref[:B * H] = ctx
        cb = ctx.astype(BF16).astype(F32)
        for b in range(B):
            for k, h in enumerate(vpu_heads):
                mul_ref[b, k * D:(k + 1) * D] = jnp.broadcast_to(cb[b * H + h:b * H + h + 1], (128, 128)).T
        with scope('d5'):
            issue_end(dcut[4], 64)

        s = jnp.zeros((B, M), F32)
        for g, hs in enumerate(mxu_heads):
            with scope('wo'):
                for h in hs:
                    wait_filled(wo_buf.at[pl.ds(8 * h, 8)], sem_o.at[g])
            lhs = jnp.concatenate([ctx_ref[pl.ds(h, B, stride=H), :] for h in hs], axis=1)
            rhs = jnp.concatenate([wo_buf[8 * h:8 * h + 8].reshape(D, M) for h in hs], axis=0)
            s = s + jnp.dot(lhs.astype(BF16), rhs, preferred_element_type=F32)
        base8 = x8 + _rows8(s) * g8

        part = [[None] * (M // 128) for _ in range(B)]
        for i, (lo, hi) in enumerate(zip((0,) + cuts, cuts)):
            with scope('wl'):
                wait_filled(wo_buf.at[pl.ds(0, hi - lo)], sem_last.at[i])
            for e in QD[256 - NV + lo:256 - NV + hi]:
                w16 = wo_buf[e].astype(F32)
                for u in range(2):
                    w = w16[8 * u:8 * u + 8]
                    r = vpu_heads.index(e // 8) * D + (e % 8) * 16 + 8 * u
                    for b in range(B):
                        mul = mul_ref[b, r:r + 8, :]
                        for j in range(M // 128):
                            t = w[:, j * 128:(j + 1) * 128] * mul
                            part[b][j] = t if part[b][j] is None else part[b][j] + t

        sl = lax.broadcasted_iota(jnp.int32, (8, 128), 0)

        def merge(lo, hi, k):
            m = (sl & k) != 0
            if k == 4:
                return jnp.where(m, hi, lo) + pltpu.roll(jnp.where(m, lo, hi), 4, 0)
            return jnp.where(m, hi, lo) + jnp.where(m, pltpu.roll(hi, k, 0), pltpu.roll(lo, 8 - k, 0))

        r4 = [[merge(part[b][j], part[b][j + 2], 4) for j in range(2)] for b in range(B)]
        r2 = [merge(r4[b][0], r4[b][1], 2) for b in range(B)]
        o_buf[...] = (base8 + g8 * merge(r2[0], r2[1], 1)).astype(BF16)
        o_copy = pltpu.make_async_copy(o_buf, o_hbm, sem_small.at[0])
        o_copy.start()
        o_copy.wait()

    def fn(A_x, A_c_kv, A_w_q, A_w_uk, A_w_uv, A_w_o, B_x, B_w1, B_b1, B_w2, B_b2):
        hbm = pl.BlockSpec(memory_space=pltpu.HBM)
        sems = pltpu.SemaphoreType.DMA
        w1_tiles = B_w1.reshape(M // 8, 8, F // 128, 128).transpose(0, 2, 1, 3).reshape(W1_VIEW)
        out = pl.pallas_call(
            kernel,
            out_shape=jax.ShapeDtypeStruct((8, 128), BF16),
            in_specs=[hbm] * 10,
            out_specs=hbm,
            scratch_shapes=[
                pltpu.VMEM((B, M), BF16), pltpu.VMEM((F,), BF16), pltpu.VMEM((M,), BF16),
                pltpu.VMEM((NBLK, 64, 16, DC), BF16), pltpu.VMEM(W_VIEW, BF16), pltpu.VMEM(W_VIEW, BF16),
                pltpu.VMEM(W_VIEW, BF16), pltpu.VMEM(O_VIEW, BF16),
                pltpu.VMEM(W1_VIEW, BF16), pltpu.VMEM(W2_VIEW, BF16),
                pltpu.VMEM((4, B * H, 128), BF16), pltpu.VMEM((B * H, DC), F32),
                pltpu.VMEM((B * H, 128), F32), pltpu.VMEM((B * H, 128), F32),
                pltpu.VMEM((4, B * H, 1024), BF16), pltpu.VMEM((128, 1024), BF16),
                pltpu.VMEM((3 * H, D), F32), pltpu.VMEM((B, len(vpu_heads) * D, 128), F32), pltpu.VMEM((8, 128), BF16),
                sems((2,)), sems((NBLK,)), sems((len(mxu_heads),)), sems((len(cuts),)), sems((3,)),
            ],
            compiler_params=pltpu.CompilerParams(
                vmem_limit_bytes=100 * 1024 * 1024, disable_semaphore_checks=True, disable_bounds_checks=True),
        )(A_x.reshape(B, M), A_c_kv.reshape(C_VIEW), A_w_q.reshape(W_VIEW), A_w_uk.reshape(W_VIEW),
          A_w_uv.reshape(W_VIEW), A_w_o.reshape(O_VIEW), w1_tiles, B_b1, B_w2.reshape(W2_VIEW), B_b2)
        return out.reshape(M // 128, B, 128).transpose(1, 0, 2).reshape(B, 1, M)
    return fn


_impl = make(**{'QA': [8, 0, 1, 9, 25, 48, 24, 49, 32, 40, 33, 41, 6, 7, 2, 10, 56, 17, 18, 59, 26, 51, 27, 50, 5, 11, 3, 4, 42, 34, 43, 35, 19, 57, 58, 15, 20, 21, 44, 45, 37, 36, 29, 28, 52, 13, 14, 16, 53, 12, 62, 63, 46, 22, 38, 30, 54, 55, 31, 39, 47, 23, 61, 60], 'QB': [30, 32, 33, 31, 27, 36, 3, 11, 10, 14, 26, 52, 34, 53, 15, 28, 29, 35, 54, 24, 12, 0, 41, 39, 8, 55, 13, 25, 9, 1, 42, 2, 37, 6, 43, 4, 16, 17, 58, 20, 46, 47, 49, 51, 38, 5, 40, 7, 18, 59, 19, 21, 50, 44, 45, 48, 22, 57, 23, 56], 'QC': [57, 56, 44, 45, 48, 52, 49, 53, 41, 40, 28, 29, 32, 33, 36, 37, 24, 25, 13, 12, 4, 0, 1, 5, 8, 20, 16, 17, 21, 9, 6, 7, 2, 3, 10, 11, 22, 23, 18, 19, 14, 15, 27, 26, 38, 34, 39, 35, 30, 61, 62, 43, 58, 47, 59, 46, 51, 50, 54, 55, 42, 63, 31, 60], 'QD': [97, 64, 65, 1, 225, 224, 192, 32, 0, 96, 33, 161, 128, 160, 68, 129, 196, 229, 195, 66, 194, 98, 2, 35, 67, 3, 165, 131, 130, 163, 100, 37, 4, 228, 197, 36, 227, 99, 226, 133, 132, 164, 162, 34, 69, 101, 5, 6, 70, 102, 198, 233, 199, 135, 169, 134, 167, 71, 38, 39, 7, 200, 103, 72, 8, 73, 136, 137, 166, 168, 104, 41, 105, 40, 9, 201, 232, 231, 230, 138, 139, 171, 75, 74, 106, 42, 43, 107, 11, 10, 193, 234, 170, 141, 235, 140, 172, 44, 108, 45, 12, 236, 202, 76, 77, 109, 13, 237, 203, 204, 173, 205, 238, 239, 14, 79, 46, 110, 15, 111, 78, 206, 142, 47, 174, 207, 175, 143, 208, 112, 241, 81, 17, 80, 240, 16, 176, 209, 177, 113, 144, 145, 48, 49, 82, 83, 18, 19, 243, 210, 179, 178, 212, 148, 114, 115, 146, 84, 20, 21, 85, 242, 51, 50, 180, 213, 181, 211, 149, 116, 147, 117, 52, 244, 245, 53, 86, 182, 22, 215, 214, 87, 23, 151, 118, 150, 247, 55, 246, 54, 183, 119, 89, 88, 216, 217, 152, 153, 25, 24, 90, 92, 91, 93, 222, 223, 28, 154, 155, 157, 26, 27, 29, 156, 95, 94, 221, 219, 218, 220, 158, 159, 31, 30, 57, 56, 120, 121, 248, 249, 185, 184, 61, 60, 125, 124, 58, 59, 123, 122, 251, 250, 252, 186, 187, 253, 188, 189, 62, 63, 126, 127, 254, 255, 191, 190]})


@jax.jit
def pallas_recurrent_scan__compressed_kv_cla__dense_activation_gelu__decode_kernel(
    A_x, A_c_kv, A_w_q, A_w_uk, A_w_uv, A_w_o, B_x, B_w1, B_b1, B_w2, B_b2,
):
    return _impl(A_x, A_c_kv, A_w_q, A_w_uk, A_w_uv, A_w_o, B_x, B_w1, B_b1, B_w2, B_b2)
```

```python
import contextlib
import jax
import jax.numpy as jnp
from jax import lax
import jax.experimental.pallas as pl
import jax.experimental.pallas.tpu as pltpu

F32 = jnp.float32
BF16 = jnp.bfloat16

B, H, SK, D, M, DC, F = 2, 32, 16384, 128, 512, 512, 1792
LOG2E = 1.4426950408889634
NT = (((1,), (1,)), ((), ()))

C_VIEW = (2048, 16, DC)
W_VIEW = (256, 2 * H, D)
O_VIEW = (256, 16, M)
W1_VIEW = (112, 64, 128)
W2_VIEW = (112, 16, M)
NBLK = 32


def _loop(lo, hi, body):
    lax.fori_loop(lo, hi, lambda i, _: body(i), None)


def _rows8(v):
    return jnp.concatenate([v[:, j * 128:(j + 1) * 128] for j in range(M // 128)], axis=0)


def natural(runs, k=None):
    k = k or len(runs)
    return [r * 4 + t for g in range(0, len(runs), k) for t in range(4) for r in runs[g:g + k]]


EVEN_ODD = [0, 2, 4, 6, 8, 10, 12, 14, 1, 3, 5, 7, 9, 11, 13, 15]
MXU_HEADS = ([4 * r + k for k in (0, 1) for r in range(8)], [4 * r + 2 for r in range(8)], [3, 11, 19, 27])
VPU_HEADS = [7, 15, 23, 31]


def order_o():
    out = []
    for heads in MXU_HEADS + (VPU_HEADS,):
        for g in range(0, len(heads), 8):
            hs = heads[g:g + 8]
            hs = hs[0::2] + hs[1::2] if len(hs) == 8 else hs
            out += [h * 8 + t for t in range(8) for h in hs]
    return out


def make(QA=None, QB=None, QC=None, QD=None, skew=(2, 2, 2, 2, 2, 3), lag=26, small=8, nsmall=4,
         cuts=(12, 20, 26, 30, 31, 32), dcut=(32, 42, 46, 50, 54), gcut=(), dma_only=False, TR=False, mxu_heads=MXU_HEADS, vpu_heads=VPU_HEADS):
    QA = QA or natural(EVEN_ODD)
    QB = QB or natural([0, 2, 4, 6, 8, 10, 11, 13, 1, 3, 5, 7, 9, 12, 14])
    QC = QC or natural(list(range(16)))
    QD = QD or order_o()
    assert sorted(QA) == sorted(QC) == list(range(64)) and sorted(QB) == list(range(60)) and sorted(QD) == list(range(256))
    NV = len(vpu_heads) * 8
    assert sorted(QD[-NV:]) == sorted(h * 8 + t for h in vpu_heads for t in range(8)) and cuts[-1] == NV
    s_c, s_q, s_k, s_v, s_1, s_2 = skew
    scope = (lambda n: jax.named_scope('@' + n)) if TR else (lambda n: contextlib.nullcontext())

    def kernel(x_hbm, ckv_hbm, wq_hbm, wuk_hbm, wuv_hbm, wo_hbm, w1_hbm, b1_hbm, w2_hbm, b2_hbm,
               o_hbm,
               x_buf, b1_buf, b2_buf, c_buf, wq_buf, wuk_buf, wuv_buf, wo_buf, w1_buf, w2_buf,
               qa_ref, acc_ref, m_ref, l_ref, a_buf, e_buf, ctx_ref, mul_ref, o_buf,
               sem_w, sem_c, sem_o, sem_last, sem_small):
        def piece(hbm, buf, i, sem):
            return pltpu.make_async_copy(hbm.at[i], buf.at[i], sem)

        def wait_filled(buf, sem):
            pltpu.make_async_copy(buf, buf, sem).wait()

        def wrap(j, last, off, n):
            i = 4 * j + off
            if 4 * last + off < n:
                return i
            return i % n if isinstance(i, int) else jnp.where(i >= n, i - n, i)

        def round_a(j):
            def one(e):
                r, t = divmod(e, 4)
                hbm, buf, s = (wq_hbm, wq_buf, s_q) if r >= 8 else (wuk_hbm, wuk_buf, s_k)
                return piece(hbm, buf, wrap(j, 7, s + (r % 8) * 32 + t, 256), sem_w.at[0])
            return [lambda e=e: one(e) for e in QA]

        def round_b(j, half):
            def one(e):
                r, t = divmod(e, 4)
                if r < 8:
                    return piece(wuv_hbm, wuv_buf, wrap(j, 7, s_v + r * 32 + t, 256), sem_w.at[1])
                if r == 14:
                    hbm, buf, s = (w2_hbm, w2_buf, s_2) if half else (w1_hbm, w1_buf, s_1)
                    return piece(hbm, buf, wrap(j, 3 + 4 * half, s + 96 - 16 * half + t, 112), sem_w.at[1])
                hbm, buf, s = (w2_hbm, w2_buf, s_2) if r >= 11 else (w1_hbm, w1_buf, s_1)
                return piece(hbm, buf, 4 * j + (s + ((r - 8) % 3) * 32 + t), sem_w.at[1])
            return [lambda e=e: one(e) for e in QB]

        def round_c(i):
            j, b = i >> 1, i & 1

            def one(e):
                r, t = divmod(e, 4)
                return pltpu.make_async_copy(ckv_hbm.at[b * 1024 + wrap(j, 15, s_c + r * 64 + t, 1024)],
                                             c_buf.at[i, e], sem_c.at[i])
            return [lambda e=e: one(e) for e in QC]

        def sem_d(n):
            if n >= 256 - NV:
                return sem_last.at[sum(n - (256 - NV) >= c for c in cuts)]
            return sem_o.at[QD[n] // 8 % 8]

        big = 256 - small
        stream_d = [lambda n=n: piece(wo_hbm, wo_buf, QD[n], sem_d(n)) for n in range(big)]

        def queue1(seq):
            return [c for n, c in enumerate(seq) if n % 4]

        def issue(cur, nxt, lo, hi, more=()):
            ones = queue1(cur + nxt) + list(more)
            for g in range(lo, min(hi, len(cur) // 4)):
                cur[4 * g]().start(priority=0)
                for c in ones[3 * g + lag:3 * g + lag + 3]:
                    c().start(priority=1)

        def issue_end(lo, hi):
            parts = []
            for n in range(big, 256):
                w = 16 * M // 8 // nsmall
                for u in range(nsmall):
                    ix = (QD[n], pl.ds(u * w // M * 8, 8), pl.ds(u * w % M, w))
                    parts.append(lambda n=n, ix=ix: pltpu.make_async_copy(wo_hbm.at[ix], wo_buf.at[ix], sem_d(n)))
            assert big % 4 == 0
            issue(stream_d, [], lo, hi, parts)
            ones = queue1(stream_d) + parts
            if hi == 64:
                for c in ones[3 * (big // 4) + lag:]:
                    c().start(priority=1)

        x_copy = pltpu.make_async_copy(x_hbm, x_buf, sem_small.at[0])
        b1_copy = pltpu.make_async_copy(b1_hbm, b1_buf, sem_small.at[1])
        b2_copy = pltpu.make_async_copy(b2_hbm, b2_buf, sem_small.at[2])

        first = round_a(0)
        first[0]().start(priority=0)
        for c in queue1(first)[:lag + 3]:
            c().start(priority=1)
        issue(first, round_a(1), 1, 16)
        for c in (x_copy, b1_copy, b2_copy):
            c.start()
        _loop(1, 4, lambda j: issue(round_a(j), round_a(j + 1), 0, 16))

        if dma_only:
            _loop(4, 7, lambda j: issue(round_a(j), round_a(j + 1), 0, 16))
            issue(round_a(7), round_b(0, 0), 0, 16)
            _loop(0, 3, lambda j: issue(round_b(j, 0), round_b(j + 1, 0), 0, 16))
            issue(round_b(3, 0), round_b(4, 1), 0, 16)
            _loop(4, 7, lambda j: issue(round_b(j, 1), round_b(j + 1, 1), 0, 16))
            issue(round_b(7, 1), round_c(0), 0, 16)
            _loop(0, 31, lambda i: issue(round_c(i), round_c(i + 1), 0, 16))
            issue(round_c(31), stream_d, 0, 16)
            issue_end(0, 64)
            for c in (x_copy, b1_copy, b2_copy):
                c.wait()
            for v in (wq_buf, wuk_buf):
                wait_filled(v, sem_w.at[0])
            for v in (wuv_buf, w1_buf, w2_buf):
                wait_filled(v, sem_w.at[1])
            for i in range(NBLK):
                wait_filled(c_buf.at[i], sem_c.at[i])
            for g in range(7):
                wait_filled(wo_buf.at[pl.ds(0, 32)], sem_o.at[g])
            for i, (lo, hi) in enumerate(zip((0,) + cuts, cuts)):
                wait_filled(wo_buf.at[pl.ds(0, hi - lo)], sem_last.at[i])
            o_copy = pltpu.make_async_copy(o_buf, o_hbm, sem_small.at[0])
            o_copy.start()
            o_copy.wait()
            return

        with scope('x'):
            x_copy.wait()
        x = x_buf[...].astype(F32)
        xc = x - jnp.mean(x, axis=-1, keepdims=True)
        var = jnp.mean(xc * xc, axis=-1, keepdims=True)
        xn = (xc * lax.rsqrt(var + 1e-5)).astype(BF16)
        e_buf[...] = (lax.broadcasted_iota(jnp.int32, (128, 1024), 1) // 8
                      == lax.broadcasted_iota(jnp.int32, (128, 1024), 0)).astype(F32).astype(BF16)
        m_ref[...] = jnp.full((B * H, 128), -jnp.inf, F32)
        l_ref[...] = jnp.zeros((B * H, 128), F32)
        acc_ref[...] = jnp.zeros((B * H, DC), F32)

        def own_head(v):
            keep = (lax.broadcasted_iota(jnp.int32, v.shape, 0) % 8 == lax.broadcasted_iota(jnp.int32, v.shape, 1) % 8)
            return jnp.where(keep, v, 0.0).astype(BF16)

        def spread(v):
            return own_head(jnp.dot(v, e_buf[...], preferred_element_type=F32))

        def heads(buf, j):
            w = buf[pl.ds(j * 64, 64)].reshape(128, 4, 8, D)
            return [w[:, g].reshape(1024, D) for g in range(4)]

        xf = xn.astype(F32)
        x16 = jnp.concatenate([jnp.broadcast_to(xf[b:b + 1], (8, M)) for b in range(B)], axis=0).astype(BF16)
        for j in range(4):
            a_buf[j, :16] = spread(x16[:, j * 128:(j + 1) * 128])
        with scope('a4'):
            _loop(4, 7, lambda j: issue(round_a(j), round_a(j + 1), 0, 16))
            issue(round_a(7), round_b(0, 0), 0, 16)

        def q_round(j, q):
            with scope('b0'):
                issue(round_b(j, 0), round_b(j + 1, 0), 0, 16)

            @pl.when(j == 1)
            def _():
                with scope('wq'):
                    wait_filled(wq_buf, sem_w.at[0])
                    wait_filled(wuk_buf, sem_w.at[0])

            def part(i, q):
                return tuple(t + jnp.dot(a_buf[i, :16], w, preferred_element_type=F32) for t, w in zip(q, heads(wq_buf, i)))
            return lax.fori_loop(jnp.maximum(2 * j - 2, 0), 2 * j, part, q)

        q = lax.fori_loop(0, 3, q_round, (jnp.zeros((16, D), F32),) * 4)
        q = [t.astype(BF16) for t in q]

        def qa_round(j):
            with scope('b3'):
                pl.when(j == 3)(lambda: issue(round_b(3, 0), round_b(4, 1), 0, 16))
                pl.when(j > 3)(lambda: issue(round_b(j, 1), round_b(j + 1, 1), 0, 16))
            r = [lax.dot_general(t, w, NT, preferred_element_type=F32) for t, w in zip(q, heads(wuk_buf, j - 3))]
            r = jnp.concatenate([t[8 * b:8 * b + 8] for b in range(B) for t in r], axis=0)
            r = own_head(r * (D ** -0.5 * LOG2E))
            qa_ref[j - 3] = lax.dot_general(r, e_buf[...], NT, preferred_element_type=F32).astype(BF16)

        _loop(3, 7, qa_round)
        with scope('b7'):
            issue(round_b(7, 1), round_c(0), 0, 16)
            _loop(0, 2, lambda i: issue(round_c(i), round_c(i + 1), 0, 16))

        with scope('w1'):
            for v in (wuv_buf, w1_buf, w2_buf):
                wait_filled(v, sem_w.at[1])
            b1_copy.wait()
            b2_copy.wait()
        w1 = w1_buf[...].reshape(M // 8, F // 128, 8, 128)
        hid = jnp.concatenate([jnp.dot(xn, w1[:, j].reshape(M, 128), preferred_element_type=F32)
                               for j in range(F // 128)], axis=1)
        hid = jax.nn.gelu(hid + b1_buf[...].astype(F32).reshape(1, F), approximate=True).astype(BF16)
        z = jnp.dot(hid, w2_buf[...].reshape(F, M), preferred_element_type=F32)
        z8 = _rows8(z + b2_buf[...].astype(F32).reshape(1, M))
        g8 = z8 * jax.nn.sigmoid(z8)
        x8 = _rows8(x)

        def feed(i, half):
            lo, hi = 8 * half, 8 * half + 8
            with scope('c'):
                pl.when(i < NBLK - 1)(lambda: issue(round_c(i), round_c(i + 1), lo, hi))
                pl.when(i == NBLK - 1)(lambda: issue(round_c(NBLK - 1), stream_d, lo, hi))
                pl.when(i == NBLK)(lambda: issue_end(lo, hi))
                pl.when(i == NBLK + 1)(lambda: issue_end(16 + lo, 16 + hi))

        def block(i):
            feed(i + 2, 0)
            with scope('wc'):
                wait_filled(c_buf.at[i], sem_c.at[i])
            hrows = pl.ds(pl.multiple_of((i & 1) * H, H), H)
            qa = jnp.concatenate([qa_ref[j, hrows] for j in range(4)], axis=1)
            sc = lax.dot_general(qa, c_buf[i].reshape(1024, DC), NT, preferred_element_type=F32)
            m_prev = m_ref[hrows, :]
            m_new = jnp.maximum(m_prev, jnp.max(sc, axis=1, keepdims=True))
            p = [jnp.exp2(sc[:, j * 128:(j + 1) * 128] - m_new) for j in range(8)]
            alpha = jnp.exp2(m_prev - m_new)
            l_ref[hrows, :] = alpha * l_ref[hrows, :] + sum(p)
            m_ref[hrows, :] = m_new
            p = jnp.concatenate(p, axis=1).astype(BF16)
            feed(i + 2, 1)
            pv = jnp.dot(p, c_buf[i].reshape(1024, DC), preferred_element_type=F32)
            acc_ref[hrows, :] = acc_ref[hrows, :] * jnp.concatenate([alpha] * 4, axis=1) + pv

        _loop(0, NBLK, block)

        pc = acc_ref[...] / jnp.sum(l_ref[...], axis=1, keepdims=True)
        pc = jnp.concatenate([pc[b * H + 8 * g:b * H + 8 * g + 8] for g in range(4) for b in range(B)], axis=0).astype(BF16)
        a = spread(jnp.concatenate([pc[:, j * 128:(j + 1) * 128] for j in range(4)], axis=0))
        a_buf[...] = a.reshape(4, B * H, 1024)

        def ctx_part(j, ctx):
            with scope('d'):
                for k, (lo, hi) in enumerate(zip(dcut[:4], dcut[1:])):
                    pl.when(j == k)(lambda: issue_end(lo, hi))
            return tuple(t + jnp.dot(a_buf[j, 16 * g:16 * g + 16], w, preferred_element_type=F32)
                         for g, (t, w) in enumerate(zip(ctx, heads(wuv_buf, j))))

        ctx = lax.fori_loop(0, 4, ctx_part, (jnp.zeros((16, D), F32),) * 4)
        ctx = jnp.concatenate([t[8 * b:8 * b + 8] for b in range(B) for t in ctx], axis=0)
        ctx_ref[:B * H] = ctx
        cb = ctx.astype(BF16).astype(F32)
        for b in range(B):
            for k, h in enumerate(vpu_heads):
                mul_ref[b, k * D:(k + 1) * D] = jnp.broadcast_to(cb[b * H + h:b * H + h + 1], (128, 128)).T

        def project(g, s):
            k = (g >> 1) + 4 * (g & 1)
            with scope('wo'):
                for r in range(4):
                    wait_filled(wo_buf.at[pl.ds(64 * r + 8 * k, 8)], sem_o.at[k])
            lhs = jnp.concatenate([ctx_ref[pl.ds(8 * r + k, B, stride=H), :] for r in range(4)], axis=1)
            rhs = jnp.concatenate([wo_buf[pl.ds(64 * r + 8 * k, 8)].reshape(D, M) for r in range(4)], axis=0)
            return s + jnp.dot(lhs.astype(BF16), rhs, preferred_element_type=F32)

        s = jnp.zeros((B, M), F32)
        for lo, hi, d0, d1 in zip((0,) + gcut, gcut + (7,), dcut[4:], dcut[5:] + (64,)):
            with scope('d5'):
                issue_end(d0, d1)
            s = lax.fori_loop(lo, hi, project, s)
        base8 = x8 + _rows8(s) * g8

        part = [[None] * (M // 128) for _ in range(B)]
        for i, (lo, hi) in enumerate(zip((0,) + cuts, cuts)):
            with scope('wl'):
                wait_filled(wo_buf.at[pl.ds(0, hi - lo)], sem_last.at[i])
            for e in QD[256 - NV + lo:256 - NV + hi]:
                w16 = wo_buf[e].astype(F32)
                for u in range(2):
                    w = w16[8 * u:8 * u + 8]
                    r = vpu_heads.index(e // 8) * D + (e % 8) * 16 + 8 * u
                    for b in range(B):
                        mul = mul_ref[b, r:r + 8, :]
                        for j in range(M // 128):
                            t = w[:, j * 128:(j + 1) * 128] * mul
                            part[b][j] = t if part[b][j] is None else part[b][j] + t

        sl = lax.broadcasted_iota(jnp.int32, (8, 128), 0)

        def merge(lo, hi, k):
            m = (sl & k) != 0
            if k == 4:
                return jnp.where(m, hi, lo) + pltpu.roll(jnp.where(m, lo, hi), 4, 0)
            return jnp.where(m, hi, lo) + jnp.where(m, pltpu.roll(hi, k, 0), pltpu.roll(lo, 8 - k, 0))

        r4 = [[merge(part[b][j], part[b][j + 2], 4) for j in range(2)] for b in range(B)]
        r2 = [merge(r4[b][0], r4[b][1], 2) for b in range(B)]
        o_buf[...] = (base8 + g8 * merge(r2[0], r2[1], 1)).astype(BF16)
        o_copy = pltpu.make_async_copy(o_buf, o_hbm, sem_small.at[0])
        o_copy.start()
        o_copy.wait()

    def fn(A_x, A_c_kv, A_w_q, A_w_uk, A_w_uv, A_w_o, B_x, B_w1, B_b1, B_w2, B_b2):
        hbm = pl.BlockSpec(memory_space=pltpu.HBM)
        sems = pltpu.SemaphoreType.DMA
        w1_tiles = B_w1.reshape(M // 8, 8, F // 128, 128).transpose(0, 2, 1, 3).reshape(W1_VIEW)
        out = pl.pallas_call(
            kernel,
            out_shape=jax.ShapeDtypeStruct((8, 128), BF16),
            in_specs=[hbm] * 10,
            out_specs=hbm,
            scratch_shapes=[
                pltpu.VMEM((B, M), BF16), pltpu.VMEM((F,), BF16), pltpu.VMEM((M,), BF16),
                pltpu.VMEM((NBLK, 64, 16, DC), BF16), pltpu.VMEM(W_VIEW, BF16), pltpu.VMEM(W_VIEW, BF16),
                pltpu.VMEM(W_VIEW, BF16), pltpu.VMEM(O_VIEW, BF16),
                pltpu.VMEM(W1_VIEW, BF16), pltpu.VMEM(W2_VIEW, BF16),
                pltpu.VMEM((4, B * H, 128), BF16), pltpu.VMEM((B * H, DC), F32),
                pltpu.VMEM((B * H, 128), F32), pltpu.VMEM((B * H, 128), F32),
                pltpu.VMEM((4, B * H, 1024), BF16), pltpu.VMEM((128, 1024), BF16),
                pltpu.VMEM((3 * H, D), F32), pltpu.VMEM((B, len(vpu_heads) * D, 128), F32), pltpu.VMEM((8, 128), BF16),
                sems((2,)), sems((NBLK,)), sems((7,)), sems((len(cuts),)), sems((3,)),
            ],
            compiler_params=pltpu.CompilerParams(
                vmem_limit_bytes=100 * 1024 * 1024, disable_semaphore_checks=True, disable_bounds_checks=True),
        )(A_x.reshape(B, M), A_c_kv.reshape(C_VIEW), A_w_q.reshape(W_VIEW), A_w_uk.reshape(W_VIEW),
          A_w_uv.reshape(W_VIEW), A_w_o.reshape(O_VIEW), w1_tiles, B_b1, B_w2.reshape(W2_VIEW), B_b2)
        return out.reshape(M // 128, B, 128).transpose(1, 0, 2).reshape(B, 1, M)
    return fn


_impl = make(**{'QA': [8, 0, 1, 9, 25, 48, 24, 49, 32, 40, 33, 41, 6, 7, 2, 10, 56, 17, 18, 59, 26, 51, 27, 50, 5, 11, 3, 4, 42, 34, 43, 35, 19, 57, 58, 15, 20, 21, 44, 45, 37, 36, 29, 28, 52, 13, 14, 16, 53, 12, 62, 63, 46, 22, 38, 30, 54, 55, 31, 39, 47, 23, 61, 60], 'QB': [30, 32, 33, 31, 27, 36, 3, 11, 10, 14, 26, 52, 34, 53, 15, 28, 29, 35, 54, 24, 12, 0, 41, 39, 8, 55, 13, 25, 9, 1, 42, 2, 37, 6, 43, 4, 16, 17, 58, 20, 46, 47, 49, 51, 38, 5, 40, 7, 18, 59, 19, 21, 50, 44, 45, 48, 22, 57, 23, 56], 'QC': [57, 56, 44, 45, 48, 52, 49, 53, 41, 40, 28, 29, 32, 33, 36, 37, 24, 25, 13, 12, 4, 0, 1, 5, 8, 20, 16, 17, 21, 9, 6, 7, 2, 3, 10, 11, 22, 23, 18, 19, 14, 15, 27, 26, 38, 34, 39, 35, 30, 61, 62, 43, 58, 47, 59, 46, 51, 50, 54, 55, 42, 63, 31, 60], 'QD': [97, 64, 65, 1, 225, 224, 192, 32, 0, 96, 33, 161, 128, 160, 68, 129, 196, 229, 195, 66, 194, 98, 2, 35, 67, 3, 165, 131, 130, 163, 100, 37, 4, 228, 197, 36, 227, 99, 226, 133, 132, 164, 162, 34, 69, 101, 5, 6, 70, 102, 198, 233, 199, 135, 169, 134, 167, 71, 38, 39, 7, 200, 103, 72, 8, 73, 136, 137, 166, 168, 104, 41, 105, 40, 9, 201, 232, 231, 230, 138, 139, 171, 75, 74, 106, 42, 43, 107, 11, 10, 193, 234, 170, 141, 235, 140, 172, 44, 108, 45, 12, 236, 202, 76, 77, 109, 13, 237, 203, 204, 173, 205, 238, 239, 14, 79, 46, 110, 15, 111, 78, 206, 142, 47, 174, 207, 175, 143, 208, 112, 241, 81, 17, 80, 240, 16, 176, 209, 177, 113, 144, 145, 48, 49, 82, 83, 18, 19, 243, 210, 179, 178, 212, 148, 114, 115, 146, 84, 20, 21, 85, 242, 51, 50, 180, 213, 181, 211, 149, 116, 147, 117, 52, 244, 245, 53, 86, 182, 22, 215, 214, 87, 23, 151, 118, 150, 247, 55, 246, 54, 183, 119, 89, 88, 216, 217, 152, 153, 25, 24, 90, 92, 91, 93, 222, 223, 28, 154, 155, 157, 26, 27, 29, 156, 95, 94, 221, 219, 218, 220, 158, 159, 31, 30, 57, 56, 120, 121, 248, 249, 185, 184, 61, 60, 125, 124, 58, 59, 123, 122, 251, 250, 252, 186, 187, 253, 188, 189, 62, 63, 126, 127, 254, 255, 191, 190], 'gcut': (2,), 'dcut': (32, 40, 44, 48, 52, 58)})


@jax.jit
def pallas_recurrent_scan__compressed_kv_cla__dense_activation_gelu__decode_kernel(
    A_x, A_c_kv, A_w_q, A_w_uk, A_w_uv, A_w_o, B_x, B_w1, B_b1, B_w2, B_b2,
):
    return _impl(A_x, A_c_kv, A_w_q, A_w_uk, A_w_uv, A_w_o, B_x, B_w1, B_b1, B_w2, B_b2)
```

```python
import contextlib
import jax
import jax.numpy as jnp
from jax import lax
import jax.experimental.pallas as pl
import jax.experimental.pallas.tpu as pltpu

F32 = jnp.float32
BF16 = jnp.bfloat16

B, H, SK, D, M, DC, F = 2, 32, 16384, 128, 512, 512, 1792
LOG2E = 1.4426950408889634
NT = (((1,), (1,)), ((), ()))

C_VIEW = (2048, 16, DC)
W_VIEW = (256, 2 * H, D)
O_VIEW = (256, 16, M)
W1_VIEW = (112, 64, 128)
W2_VIEW = (112, 16, M)


def _loop(lo, hi, body):
    lax.fori_loop(lo, hi, lambda i, _: body(i), None)


def _rows8(v):
    return jnp.concatenate([v[:, j * 128:(j + 1) * 128] for j in range(M // 128)], axis=0)


def make(QA=tuple(range(64)), QB=tuple(range(60)), QC=tuple(range(128)), QD=tuple(range(32)), QE=None,
         QM=(5, 5, 5, 4, 4, 1, 1, 0), skew=(46, 14, 14, 15), lag=26, ph=0, end='qqqqqq11',
         cuts=(12, 20, 26, 30, 31, 32), dcut=(22, 30, 38, 48, 56, 64), gcut=(0, 2, 4), TR=False, tail=0):
    QE = QE or QD
    assert sorted(QA) == list(range(64)) and sorted(QB) == list(range(60)) and sorted(QC) == list(range(128))
    assert sorted(QD) == sorted(QE) == list(range(32)) and cuts[-1] == 32 and len(end) % 4 == 0
    s_c, s_w, s_1, s_2 = skew
    scope = (lambda n: jax.named_scope('@' + n)) if TR else (lambda n: contextlib.nullcontext())

    def kernel(x_hbm, ckv_hbm, wq_hbm, wuk_hbm, wuv_hbm, wo_hbm, w1_hbm, b1_hbm, w2_hbm, b2_hbm,
               o_hbm,
               x_buf, b1_buf, b2_buf, c_buf, wq_buf, wuk_buf, wuv_buf, wo_buf, w1_buf, w2_buf,
               qa_ref, acc_ref, m_ref, l_ref, a_buf, e_buf, ctx_ref, lhs_ref, mul_ref, o_buf,
               sems):
        S_C, S_O, S_LAST, S_SMALL = 2, 18, 25, 25 + len(cuts)

        def wait_filled(buf, sem):
            pltpu.make_async_copy(buf, buf, sem).wait()

        def wrap(j, last, off, n):
            off %= n
            i = 4 * j + off
            if 4 * last + off < n:
                return i
            return i % n if isinstance(i, int) else jnp.where(i >= n, i - n, i)

        def same(hbm, buf, i, sem):
            return hbm.at[i], buf.at[i], sem

        def round_a(j):
            def one(e):
                r, t = divmod(e, 4)
                hbm, buf = (wq_hbm, wq_buf) if r >= 8 else (wuk_hbm, wuk_buf)
                return same(hbm, buf, wrap(j, 7, s_w + (r % 8) * 32 + t, 256), sems.at[0])
            return [lambda e=e: one(e) for e in QA]

        def round_b(j, half):
            def one(e):
                r, t = divmod(e, 4)
                if r < 8:
                    return same(wuv_hbm, wuv_buf, wrap(j, 7, s_w + r * 32 + t, 256), sems.at[1])
                if r == 14:
                    hbm, buf, s = (w2_hbm, w2_buf, s_2) if half else (w1_hbm, w1_buf, s_1)
                    return same(hbm, buf, wrap(j - 4 * half, 3, s + 96 + t, 112), sems.at[1])
                hbm, buf, s = (w2_hbm, w2_buf, s_2) if r >= 11 else (w1_hbm, w1_buf, s_1)
                return same(hbm, buf, wrap(j, 7, s + ((r - 8) % 3) * 32 + t, 112), sems.at[1])
            return [lambda e=e: one(e) for e in QB]

        def round_c(j):
            def one(e):
                b, r, t = e // 64, e // 4 % 16, e % 4
                return ckv_hbm.at[b * 1024 + wrap(j, 15, s_c + r * 64 + t, 1024)], c_buf.at[j, e], sems.at[S_C + j]
            return [lambda e=e: one(e) for e in QC]

        def round_d(j):
            last = isinstance(j, int) and j == 7

            def one(n, e):
                r, t = divmod(e, 4)
                sem = sems.at[S_LAST + sum(n >= c for c in cuts)] if last else sems.at[S_O + j]
                return wo_hbm.at[wrap(j ^ QM[r], 7, s_w + r * 32 + t, 256)], wo_buf.at[j, n if last else e], sem
            return [lambda n=n, e=e: one(n, e) for n, e in enumerate(QE if last else QD)]

        def start(piece, queue):
            pltpu.make_async_copy(*piece()).start(priority=queue)

        def queue1(seq):
            return [c for n, c in enumerate(seq) if n % 4 != ph]

        def issue(cur, nxt, lo=0, hi=64, more=()):
            ones = queue1(cur + nxt) + list(more)
            for g in range(lo, min(hi, len(cur) // 4)):
                start(cur[4 * g + ph], 0)
                for c in ones[3 * g + ph + lag:3 * g + ph + lag + 3]:
                    start(c, 1)

        def issue_end(lo, hi):
            seq = sum((round_d(j) for j in range(8)), [])
            big = 256 - len(end)
            parts = []
            for c, kind in zip(seq[big:], end):
                n = {'q': 4, 'h': 2, '1': 1}[kind]
                for u in range(n):
                    ix = {4: (pl.ds(u // 2 * 8, 8), pl.ds(u % 2 * 256, 256)), 2: pl.ds(u * 8, 8), 1: slice(None)}[n]
                    parts.append(lambda c=c, ix=ix: (lambda s, d, sem: (s.at[ix], d.at[ix], sem))(*c()))
            issue(seq[:big], [], lo, hi, parts)
            if hi == 64:
                for c in (queue1(seq[:big]) + parts)[3 * (big // 4) + ph + lag:]:
                    start(c, 1)

        x_copy = pltpu.make_async_copy(x_hbm, x_buf, sems.at[S_SMALL + 0])
        b1_copy = pltpu.make_async_copy(b1_hbm, b1_buf, sems.at[S_SMALL + 1])
        b2_copy = pltpu.make_async_copy(b2_hbm, b2_buf, sems.at[S_SMALL + 2])

        first = round_a(0)
        for n, c in enumerate(queue1(first)[:ph + lag + 3]):
            if n == ph:
                start(first[ph], 0)
            start(c, 1)
        issue(first, round_a(1), 1)
        for c in (x_copy, b1_copy, b2_copy):
            c.start()
        _loop(1, 4, lambda j: issue(round_a(j), round_a(j + 1)))

        with scope('x'):
            x_copy.wait()
        x = x_buf[...].astype(F32)
        xc = x - jnp.mean(x, axis=-1, keepdims=True)
        var = jnp.mean(xc * xc, axis=-1, keepdims=True)
        xn = (xc * lax.rsqrt(var + 1e-5)).astype(BF16)
        e_buf[...] = (lax.broadcasted_iota(jnp.int32, (128, 1024), 1) // 8
                      == lax.broadcasted_iota(jnp.int32, (128, 1024), 0)).astype(F32).astype(BF16)
        m_ref[...] = jnp.full((B * H, 128), -jnp.inf, F32)
        l_ref[...] = jnp.zeros((B * H, 128), F32)
        acc_ref[...] = jnp.zeros((B * H, DC), F32)

        def own_head(v):
            keep = (lax.broadcasted_iota(jnp.int32, v.shape, 0) % 8 == lax.broadcasted_iota(jnp.int32, v.shape, 1) % 8)
            return jnp.where(keep, v, 0.0).astype(BF16)

        def spread(v):
            return own_head(jnp.dot(v, e_buf[...], preferred_element_type=F32))

        def heads(buf, j):
            w = buf[pl.ds(j * 64, 64)].reshape(128, 4, 8, D)
            return [w[:, g].reshape(1024, D) for g in range(4)]

        xf = xn.astype(F32)
        x16 = jnp.concatenate([jnp.broadcast_to(xf[b:b + 1], (8, M)) for b in range(B)], axis=0).astype(BF16)
        for j in range(4):
            a_buf[j, :16] = spread(x16[:, j * 128:(j + 1) * 128])
        with scope('a4'):
            _loop(4, 7, lambda j: issue(round_a(j), round_a(j + 1)))
            issue(round_a(7), round_b(0, 0))
            issue(round_b(0, 0), round_b(1, 0))
            issue(round_b(1, 0), round_b(2, 0), 0, 8)

        with scope('wq'):
            wait_filled(wq_buf, sems.at[0])
            wait_filled(wuk_buf, sems.at[0])

        def q_part(i, q):
            with scope('b1'):
                pl.when(i == 2)(lambda: issue(round_b(1, 0), round_b(2, 0), 8))
            return tuple(t + jnp.dot(a_buf[i, :16], w, preferred_element_type=F32) for t, w in zip(q, heads(wq_buf, i)))

        q = lax.fori_loop(0, 4, q_part, (jnp.zeros((16, D), F32),) * 4)
        q = [t.astype(BF16) for t in q]

        def qa_part(i):
            with scope('b3'):
                pl.when(i == 0)(lambda: issue(round_b(2, 0), round_b(3, 0)))
                pl.when(i == 1)(lambda: issue(round_b(3, 0), round_c(0)))
                pl.when(i == 2)(lambda: issue(round_c(0), round_c(1), 0, 16))
                pl.when(i == 3)(lambda: issue(round_c(0), round_c(1), 16))
            r = [lax.dot_general(t, w, NT, preferred_element_type=F32) for t, w in zip(q, heads(wuk_buf, i))]
            r = jnp.concatenate([t[8 * b:8 * b + 8] for b in range(B) for t in r], axis=0)
            r = own_head(r * (D ** -0.5 * LOG2E))
            qa_ref[i] = lax.dot_general(r, e_buf[...], NT, preferred_element_type=F32).astype(BF16)

        _loop(0, 4, qa_part)
        with scope('c1'):
            issue(round_c(1), round_c(2), 0, 16)

        def feed(j, k):
            lo, hi = 8 * k, 8 * k + 8
            with scope('c'):
                pl.when(j < 15)(lambda: issue(round_c(j), round_c(j + 1), lo, hi))
                pl.when(j == 15)(lambda: issue(round_c(15), round_b(4, 1), lo, hi))
                n = 4 + (j - 16) * 2 + k // 2
                pl.when(j > 15)(lambda: issue(round_b(n, 1), round_b(n + 1, 1), lo % 16, lo % 16 + 8))

        def block(j):
            for b in range(B):
                feed(j + 1 + b, 2 - 2 * b)
                if b == 0:
                    with scope('wc'):
                        wait_filled(c_buf.at[j], sems.at[S_C + j])
                hrows = pl.ds(b * H, H)
                keys = (j, pl.ds(b * 64, 64))
                qa = jnp.concatenate([qa_ref[i, hrows] for i in range(4)], axis=1)
                sc = lax.dot_general(qa, c_buf[keys].reshape(1024, DC), NT, preferred_element_type=F32)
                m_prev = m_ref[hrows, :]
                m_new = jnp.maximum(m_prev, jnp.max(sc, axis=1, keepdims=True))
                p = [jnp.exp2(sc[:, i * 128:(i + 1) * 128] - m_new) for i in range(8)]
                alpha = jnp.exp2(m_prev - m_new)
                l_ref[hrows, :] = alpha * l_ref[hrows, :] + sum(p)
                m_ref[hrows, :] = m_new
                p = jnp.concatenate(p, axis=1).astype(BF16)
                feed(j + 1 + b, 3 - 2 * b)
                pv = jnp.dot(p, c_buf[keys].reshape(1024, DC), preferred_element_type=F32)
                acc_ref[hrows, :] = acc_ref[hrows, :] * jnp.concatenate([alpha] * 4, axis=1) + pv

        _loop(0, 16, block)

        pc = acc_ref[...] / jnp.sum(l_ref[...], axis=1, keepdims=True)
        pc = jnp.concatenate([pc[b * H + 8 * g:b * H + 8 * g + 8] for g in range(4) for b in range(B)], axis=0).astype(BF16)
        a = spread(jnp.concatenate([pc[:, j * 128:(j + 1) * 128] for j in range(4)], axis=0))
        a_buf[...] = a.reshape(4, B * H, 1024)

        with scope('b7'):
            issue(round_b(7, 1), round_d(0) + round_d(1))
            issue_end(0, dcut[0])
        with scope('w1'):
            for v in (wuv_buf, w1_buf, w2_buf):
                wait_filled(v, sems.at[1])
            b1_copy.wait()
            b2_copy.wait()

        def ctx_part(j, ctx):
            with scope('d'):
                pl.when(j == 2)(lambda: issue_end(dcut[0], dcut[1]))
            return tuple(t + jnp.dot(a_buf[j, 16 * g:16 * g + 16], w, preferred_element_type=F32)
                         for g, (t, w) in enumerate(zip(ctx, heads(wuv_buf, j))))

        ctx = lax.fori_loop(0, 4, ctx_part, (jnp.zeros((16, D), F32),) * 4)
        with scope('d1'):
            issue_end(dcut[1], dcut[2])
        ctx_ref[:B * H] = jnp.concatenate([t[8 * b:8 * b + 8] for b in range(B) for t in ctx], axis=0).astype(BF16).astype(F32)
        flat = jnp.concatenate([ctx_ref[pl.ds(h % H, B, stride=H), :] for h in range(H + 1)], axis=1)
        for j in reversed(range(8)):
            k0 = [(s_w + r * 32 + (j ^ QM[r]) * 4) % 256 * 16 for r in range(8)]
            lhs_ref[j] = jnp.concatenate([flat[:, k:k + 64] for k in k0], axis=1)
        for b in range(B):
            for k in range(4):
                mul_ref[b, k * D:(k + 1) * D] = jnp.broadcast_to(lhs_ref[7, b:b + 1, k * D:(k + 1) * D], (128, 128)).T

        w1 = w1_buf[...].reshape(M // 8, F // 128, 8, 128)
        hid = jnp.concatenate([jnp.dot(xn, w1[:, j].reshape(M, 128), preferred_element_type=F32)
                               for j in range(F // 128)], axis=1)
        hid = jax.nn.gelu(hid + b1_buf[...].astype(F32).reshape(1, F), approximate=True).astype(BF16)
        z = jnp.dot(hid, w2_buf[...].reshape(F, M), preferred_element_type=F32)
        z8 = _rows8(z + b2_buf[...].astype(F32).reshape(1, M))
        g8 = z8 * jax.nn.sigmoid(z8)
        x8 = _rows8(x)

        def project(j, s):
            with scope('wo'):
                for k, lo, hi in zip(gcut, dcut[2:], dcut[3:]):
                    pl.when(j == k)(lambda: issue_end(lo, hi))
                wait_filled(wo_buf.at[j], sems.at[S_O + j])
            return s + jnp.dot(lhs_ref[j].astype(BF16), wo_buf[j].reshape(512, M), preferred_element_type=F32)

        s = lax.fori_loop(0, 7, project, jnp.zeros((B, M), F32))
        base8 = x8 + _rows8(s) * g8

        part = [[None] * (M // 128) for _ in range(B)]
        for i, (lo, hi) in enumerate(zip((0,) + cuts, cuts)):
            with scope('wl'):
                wait_filled(wo_buf.at[7, pl.ds(lo, hi - lo)], sems.at[S_LAST + i])
            for n in range(lo, hi):
                w16 = wo_buf[7, n].astype(F32)
                for u in range(2):
                    w = w16[8 * u:8 * u + 8]
                    r = QE[n] * 16 + 8 * u
                    for b in range(B):
                        mul = mul_ref[b, r:r + 8, :]
                        for j in range(M // 128):
                            t = w[:, j * 128:(j + 1) * 128] * mul
                            part[b][j] = t if part[b][j] is None else part[b][j] + t

        sl = lax.broadcasted_iota(jnp.int32, (8, 128), 0)

        def merge(lo, hi, k):
            m = (sl & k) != 0
            if k == 4:
                return jnp.where(m, hi, lo) + pltpu.roll(jnp.where(m, lo, hi), 4, 0)
            return jnp.where(m, hi, lo) + jnp.where(m, pltpu.roll(hi, k, 0), pltpu.roll(lo, 8 - k, 0))

        r4 = [[merge(part[b][j], part[b][j + 2], 4) for j in range(2)] for b in range(B)]
        r2 = [merge(r4[b][0], r4[b][1], 2) for b in range(B)]
        o_buf[...] = (base8 + g8 * merge(r2[0], r2[1], 1)).astype(BF16)
        o_copy = pltpu.make_async_copy(o_buf, o_hbm, sems.at[S_SMALL + 0])
        o_copy.start()
        o_copy.wait()

    def fn(A_x, A_c_kv, A_w_q, A_w_uk, A_w_uv, A_w_o, B_x, B_w1, B_b1, B_w2, B_b2):
        hbm = pl.BlockSpec(memory_space=pltpu.HBM)
        sems = pltpu.SemaphoreType.DMA
        w1_tiles = B_w1.reshape(M // 8, 8, F // 128, 128).transpose(0, 2, 1, 3).reshape(W1_VIEW)
        out = pl.pallas_call(
            kernel,
            out_shape=jax.ShapeDtypeStruct((8, 128), BF16),
            in_specs=[hbm] * 10,
            out_specs=hbm,
            scratch_shapes=[
                pltpu.VMEM((B, M), BF16), pltpu.VMEM((F,), BF16), pltpu.VMEM((M,), BF16),
                pltpu.VMEM((16, 128, 16, DC), BF16), pltpu.VMEM(W_VIEW, BF16), pltpu.VMEM(W_VIEW, BF16),
                pltpu.VMEM(W_VIEW, BF16), pltpu.VMEM((8, 32, 16, M), BF16),
                pltpu.VMEM(W1_VIEW, BF16), pltpu.VMEM(W2_VIEW, BF16),
                pltpu.VMEM((4, B * H, 128), BF16), pltpu.VMEM((B * H, DC), F32),
                pltpu.VMEM((B * H, 128), F32), pltpu.VMEM((B * H, 128), F32),
                pltpu.VMEM((4, B * H, 1024), BF16), pltpu.VMEM((128, 1024), BF16),
                pltpu.VMEM((3 * H, D), F32), pltpu.VMEM((8, B, 512), F32), pltpu.VMEM((B, 512, 128), F32),
                pltpu.VMEM((8, 128), BF16),
                sems((28 + len(cuts),)),
            ],
            compiler_params=pltpu.CompilerParams(
                vmem_limit_bytes=100 * 1024 * 1024, disable_semaphore_checks=True, disable_bounds_checks=True),
        )(A_x.reshape(B, M), A_c_kv.reshape(C_VIEW), A_w_q.reshape(W_VIEW), A_w_uk.reshape(W_VIEW),
          A_w_uv.reshape(W_VIEW), A_w_o.reshape(O_VIEW), w1_tiles, B_b1, B_w2.reshape(W2_VIEW), B_b2)
        return out.reshape(M // 128, B, 128).transpose(1, 0, 2).reshape(B, 1, M)
    return fn


_impl = make(**{'QA': [44, 20, 45, 21, 52, 36, 60, 5, 28, 37, 29, 13, 55, 14, 61, 4, 47, 23, 22, 46, 62, 63, 39, 38, 15, 53, 54, 59, 31, 30, 7, 6, 12, 18, 17, 56, 33, 41, 32, 40, 48, 24, 25, 49, 16, 0, 8, 1, 9, 57, 58, 19, 43, 35, 42, 34, 50, 26, 51, 27, 10, 2, 3, 11], 'QB': [16, 13, 43, 42, 5, 4, 29, 15, 17, 28, 34, 35, 3, 2, 18, 12, 10, 40, 7, 41, 19, 14, 30, 6, 1, 32, 31, 33, 44, 50, 20, 26, 0, 8, 39, 9, 25, 23, 49, 47, 55, 58, 54, 56, 46, 24, 51, 21, 38, 11, 37, 36, 22, 27, 45, 48, 57, 53, 59, 52], 'QC': [24, 69, 37, 56, 16, 48, 45, 13, 21, 53, 40, 8, 29, 32, 64, 125, 61, 0, 36, 25, 57, 68, 1, 60, 28, 33, 65, 124, 44, 12, 17, 49, 41, 20, 9, 52, 30, 35, 67, 126, 62, 3, 70, 59, 38, 27, 2, 63, 5, 31, 34, 6, 10, 55, 42, 23, 46, 14, 19, 51, 7, 127, 66, 4, 11, 43, 54, 22, 50, 18, 15, 47, 87, 75, 86, 74, 78, 82, 83, 79, 71, 58, 26, 39, 103, 90, 122, 121, 117, 85, 72, 104, 112, 80, 77, 109, 92, 96, 93, 97, 89, 100, 88, 101, 108, 76, 81, 113, 105, 73, 84, 116, 120, 102, 91, 123, 98, 94, 95, 99, 114, 110, 115, 111, 119, 107, 106, 118], 'QD': [30, 29, 28, 31, 14, 7, 16, 3, 24, 13, 6, 25, 18, 17, 12, 5, 2, 11, 10, 19, 20, 1, 26, 15, 4, 27, 0, 9, 8, 23, 22, 21], 'ph': 1, 'cuts': (12, 20, 24, 27, 29, 30, 31, 32)})


@jax.jit
def pallas_recurrent_scan__compressed_kv_cla__dense_activation_gelu__decode_kernel(
    A_x, A_c_kv, A_w_q, A_w_uk, A_w_uv, A_w_o, B_x, B_w1, B_b1, B_w2, B_b2,
):
    return _impl(A_x, A_c_kv, A_w_q, A_w_uk, A_w_uv, A_w_o, B_x, B_w1, B_b1, B_w2, B_b2)
```

```python
import jax
import jax.numpy as jnp
from jax import lax
import jax.experimental.pallas as pl
import jax.experimental.pallas.tpu as pltpu

F32 = jnp.float32
BF16 = jnp.bfloat16

B, H, SK, D, M, DC, F = 2, 32, 16384, 128, 512, 512, 1792
LOG2E = 1.4426950408889634
NN = (((1,), (0,)), ((), ()))
NT = (((1,), (1,)), ((), ()))

C_VIEW = (B * SK // 16, 16, DC)
W_VIEW = (M // 2, 2 * H, D)
O_VIEW = (H * D // 16, 16, M)
W1_VIEW = (F // 16, 64, 128)
W2_VIEW = (F // 16, 16, M)

ORDER_QK = (52, 13, 14, 55, 61, 60, 36, 37, 28, 29, 5, 4, 15, 54, 53, 12, 62, 63, 39, 38, 31, 30, 6, 7, 19,
            58, 57, 16, 40, 33, 41, 32, 49, 24, 47, 22, 0, 8, 9, 1, 23, 46, 48, 25, 56, 17, 18, 59, 34, 43,
            35, 42, 45, 20, 51, 26, 50, 27, 21, 44, 2, 10, 3, 11)
ORDER_VF = ((36, 37, 42, 4, 17, 12, 19, 13, 29, 28, 35, 34, 43, 5, 38, 39, 14, 16, 15, 18, 2, 41, 6, 11, 33,
             31, 32, 30, 7, 3, 10, 40, 20, 26, 22, 27, 45, 51, 50, 47, 8, 0, 9, 1, 52, 58, 59, 54, 24, 21,
             25, 23, 44, 49, 46, 48, 53, 56, 57, 55),
            (12, 17, 42, 16, 0, 29, 36, 28, 55, 54, 53, 43, 15, 18, 41, 52, 1, 37, 30, 6, 14, 19, 13, 40, 7,
             31, 2, 38, 27, 21, 26, 23, 11, 5, 32, 3, 44, 51, 59, 50, 39, 10, 4, 33, 20, 25, 22, 24, 58, 47,
             49, 45, 35, 8, 34, 9, 48, 57, 46, 56))
ORDER_C = (58, 36, 71, 25, 127, 33, 66, 28, 16, 12, 17, 13, 52, 9, 20, 41, 125, 64, 32, 29, 61, 1, 0, 60,
           7, 65, 124, 4, 8, 40, 21, 53, 117, 85, 72, 104, 92, 96, 93, 97, 116, 84, 73, 105, 113, 81, 76,
           108, 6, 34, 31, 5, 44, 45, 48, 49, 112, 80, 77, 109, 69, 56, 37, 24, 55, 23, 42, 10, 101, 88,
           89, 100, 2, 63, 57, 68, 50, 15, 18, 47, 26, 39, 3, 62, 126, 67, 35, 30, 59, 38, 70, 27, 22, 54,
           11, 43, 19, 51, 14, 46, 110, 78, 83, 115, 75, 107, 118, 86, 111, 79, 82, 114, 123, 91, 102, 120,
           74, 106, 119, 87, 94, 99, 95, 98, 121, 90, 103, 122)
ORDER_O = (30, 29, 28, 31, 14, 7, 16, 3, 24, 13, 6, 25, 18, 17, 12, 5, 2, 11, 10, 19, 20, 1, 26, 15, 4,
           27, 0, 9, 8, 23, 22, 21)
FLIP_O = (5, 5, 5, 4, 4, 1, 1, 0)
SKEW_C, SKEW_W, SKEW_W2 = 46, 14, 15
LAG = 26
HALVED = 12
LAST_CUTS = (0, 192, 320, 384, 432, 464, 480, 496, 512)
GATED = 3

C_ROUNDS = 16
S_Q, S_K, S_V, S_W1, S_W2, S_X, S_B1, S_B2, S_OUT, S_C = range(10)
S_O = S_C + C_ROUNDS
S_LAST = S_O + 7


def _loop(lo, hi, body):
    lax.fori_loop(lo, hi, lambda i, _: body(i), None)


def _dot(a, b, dims=NN):
    return lax.dot_general(a, b, dims, preferred_element_type=F32)


def _iota(shape, axis):
    return lax.broadcasted_iota(jnp.int32, shape, axis)


def _piece(j, rounds, first, n):
    first %= n
    i = first + 4 * j
    if first + 4 * (rounds - 1) < n:
        return i
    return i % n if isinstance(i, int) else jnp.where(i >= n, i - n, i)


def _kernel(x_hbm, ckv_hbm, wq_hbm, wuk_hbm, wuv_hbm, wo_hbm, w1_hbm, b1_hbm, w2_hbm, b2_hbm,
            o_hbm,
            c_buf, wq_buf, wuk_buf, wuv_buf, wo_buf, w1_buf, w2_buf,
            qa_ref, acc_ref, m_ref, l_ref, a_buf, e_buf, ctx_ref, lhs_ref, mul_ref, gmul_ref,
            o_buf, x_buf, b1_buf, b2_buf, sems):
    def round_qk(j):
        def one(r, t):
            hbm, buf, sem = (wq_hbm, wq_buf, S_Q) if r >= 8 else (wuk_hbm, wuk_buf, S_K)
            i = _piece(j, 8, SKEW_W + r % 8 * 32 + t, 256)
            return hbm.at[i], buf.at[i], sem
        return [lambda e=e: one(*divmod(e, 4)) for e in ORDER_QK]

    def round_vf(half, j):
        def one(r, t):
            if r < 8:
                i = _piece(j, 4, SKEW_W + r * 32 + half * 16 + t, 256)
                return wuv_hbm.at[i], wuv_buf.at[i], S_V
            second = half if r == 14 else r >= 11
            hbm, buf, sem, skew = (w2_hbm, w2_buf, S_W2, SKEW_W2) if second else (w1_hbm, w1_buf, S_W1, SKEW_W)
            i = _piece(j, 4, skew + (96 if r == 14 else (r - 8) % 3 * 32 + half * 16) + t, 112)
            return hbm.at[i], buf.at[i], sem
        return [lambda e=e: one(*divmod(e, 4)) for e in ORDER_VF[half]]

    def round_c(j):
        def one(r, t):
            i = r // 16 * 1024 + _piece(j, C_ROUNDS, SKEW_C + r % 16 * 64 + t, 1024)
            return ckv_hbm.at[i], c_buf.at[j, 4 * r + t], S_C + j
        return [lambda e=e: one(*divmod(e, 4)) for e in ORDER_C]

    def piece_o(n, lo=0, hi=16):
        j, e = n // 32, ORDER_O[n % 32]
        i = _piece(j ^ FLIP_O[e // 4], 8, SKEW_W + e // 4 * 32 + e % 4, 256)
        row = 16 * (e if j < 7 else n % 32)
        sem = S_O + j if j < 7 else S_LAST + sum(row >= c for c in LAST_CUTS[1:])
        return wo_hbm.at[i, lo:hi], wo_buf.at[j, row + lo:row + hi], sem

    stream_o = [lambda n=n: piece_o(n) for n in range(256 - HALVED)]
    halves_o = [lambda n=n, r=r: piece_o(n, r, r + 8) for n in range(256 - HALVED, 256) for r in (0, 8)]

    def start(piece, queue):
        src, dst, sem = piece()
        pltpu.make_async_copy(src, dst, sems.at[sem]).start(priority=queue)

    def queue1(pieces):
        return [p for n, p in enumerate(pieces) if n % 4 != 1]

    def issue(cur, nxt, lo=0, hi=64, end=()):
        ahead = (queue1(cur + nxt) + list(end))[LAG + 1:]
        for g in range(lo, min(hi, len(cur) // 4)):
            start(cur[4 * g + 1], 0)
            for p in ahead[3 * g:3 * g + 3]:
                start(p, 1)

    def issue_o(lo, hi):
        issue(stream_o, [], lo, hi, halves_o)

    def wait_filled(buf, sem):
        pltpu.make_async_copy(buf, buf, sems.at[sem]).wait()

    first = round_qk(0)
    start(first[0], 1)
    start(first[1], 0)
    for p in queue1(first)[1:LAG + 4]:
        start(p, 1)
    issue(first, round_qk(1), 1)
    for hbm, buf, sem in ((x_hbm, x_buf, S_X), (b1_hbm, b1_buf, S_B1), (b2_hbm, b2_buf, S_B2)):
        pltpu.make_async_copy(hbm, buf, sems.at[sem]).start()
    _loop(1, 4, lambda j: issue(round_qk(j), round_qk(j + 1)))

    pltpu.make_async_copy(x_hbm, x_buf, sems.at[S_X]).wait()
    x = x_buf[...].astype(F32)
    xc = x - jnp.mean(x, axis=-1, keepdims=True)
    var = jnp.mean(xc * xc, axis=-1, keepdims=True)
    xn = (xc * lax.rsqrt(var + 1e-5)).astype(BF16)

    e_buf[...] = (_iota((128, 1024), 1) // 8 == _iota((128, 1024), 0)).astype(F32).astype(BF16)

    def own_head(v):
        return jnp.where(_iota(v.shape, 0) % 8 == _iota(v.shape, 1) % 8, v, 0.0).astype(BF16)

    def heads(buf, i):
        w = buf[pl.ds(i * 64, 64)].reshape(128, 4, 8, D)
        return [w[:, g].reshape(1024, D) for g in range(4)]

    def by_batch(groups):
        return jnp.concatenate([t[8 * b:8 * b + 8] for b in range(B) for t in groups], axis=0)

    xf = xn.astype(F32)
    x16 = jnp.concatenate([jnp.broadcast_to(xf[b:b + 1], (8, M)) for b in range(B)], axis=0).astype(BF16)
    for i in range(4):
        a_buf[i, :16] = own_head(_dot(x16[:, i * 128:(i + 1) * 128], e_buf[...]))
    m_ref[...] = jnp.full((B * H, 128), -jnp.inf, F32)
    l_ref[...] = jnp.zeros((B * H, 128), F32)
    acc_ref[...] = jnp.zeros((B * H, DC), F32)
    _loop(4, 7, lambda j: issue(round_qk(j), round_qk(j + 1)))
    issue(round_qk(7), round_vf(0, 0))
    issue(round_vf(0, 0), round_vf(0, 1))
    issue(round_vf(0, 1), round_vf(0, 2), 0, 8)

    wait_filled(wq_buf, S_Q)
    wait_filled(wuk_buf, S_K)

    def q_part(i, q):
        pl.when(i == 2)(lambda: issue(round_vf(0, 1), round_vf(0, 2), 8))
        return tuple(t + _dot(a_buf[i, :16], w) for t, w in zip(q, heads(wq_buf, i)))

    q = [t.astype(BF16) for t in lax.fori_loop(0, 4, q_part, (jnp.zeros((16, D), F32),) * 4)]

    def qa_part(i):
        pl.when(i == 0)(lambda: issue(round_vf(0, 2), round_vf(0, 3)))
        pl.when(i == 1)(lambda: issue(round_vf(0, 3), round_c(0)))
        pl.when(i == 2)(lambda: issue(round_c(0), round_c(1), 0, 16))
        pl.when(i == 3)(lambda: issue(round_c(0), round_c(1), 16))
        r = by_batch([_dot(t, w, NT) for t, w in zip(q, heads(wuk_buf, i))])
        qa_ref[i] = _dot(own_head(r * (D ** -0.5 * LOG2E)), e_buf[...], NT).astype(BF16)

    _loop(0, 4, qa_part)
    issue(round_c(1), round_c(2), 0, 16)

    def feed(j, k):
        last = C_ROUNDS - 1
        pl.when(j < last)(lambda: issue(round_c(j), round_c(j + 1), 8 * k, 8 * k + 8))
        pl.when(j == last)(lambda: issue(round_c(last), round_vf(1, 0), 8 * k, 8 * k + 8))
        n = (j - C_ROUNDS) * 2 + k // 2
        pl.when(j > last)(lambda: issue(round_vf(1, n), round_vf(1, n + 1), k % 2 * 8, k % 2 * 8 + 8))

    def block(j):
        for b in range(B):
            feed(j + 1 + b, 2 - 2 * b)
            if b == 0:
                wait_filled(c_buf.at[j], S_C + j)
            rows = pl.ds(b * H, H)
            keys = (j, pl.ds(b * 64, 64))
            qa = jnp.concatenate([qa_ref[i, rows] for i in range(4)], axis=1)
            sc = _dot(qa, c_buf[keys].reshape(1024, DC), NT)
            m_prev = m_ref[rows, :]
            m_new = jnp.maximum(m_prev, jnp.max(sc, axis=1, keepdims=True))
            p = [jnp.exp2(sc[:, i * 128:(i + 1) * 128] - m_new) for i in range(8)]
            alpha = jnp.exp2(m_prev - m_new)
            l_ref[rows, :] = alpha * l_ref[rows, :] + sum(p)
            m_ref[rows, :] = m_new
            p = jnp.concatenate(p, axis=1).astype(BF16)
            feed(j + 1 + b, 3 - 2 * b)
            pv = _dot(p, c_buf[keys].reshape(1024, DC))
            acc_ref[rows, :] = acc_ref[rows, :] * jnp.concatenate([alpha] * 4, axis=1) + pv

    _loop(0, C_ROUNDS, block)

    pc = acc_ref[...] / jnp.sum(l_ref[...], axis=1, keepdims=True)
    pc = jnp.concatenate([pc[b * H + 8 * g:b * H + 8 * g + 8, i * 128:(i + 1) * 128]
                          for i in range(4) for g in range(4) for b in range(B)], axis=0)
    a_buf[...] = own_head(_dot(pc.astype(BF16), e_buf[...])).reshape(4, B * H, 1024)
    issue(round_vf(1, 3), stream_o)
    issue_o(0, 22)
    wait_filled(wuv_buf, S_V)
    wait_filled(w1_buf, S_W1)
    wait_filled(w2_buf, S_W2)
    pltpu.make_async_copy(b1_hbm, b1_buf, sems.at[S_B1]).wait()
    pltpu.make_async_copy(b2_hbm, b2_buf, sems.at[S_B2]).wait()

    def ctx_part(i, ctx):
        pl.when(i == 2)(lambda: issue_o(22, 30))
        return tuple(t + _dot(a_buf[i, 16 * g:16 * g + 16], w)
                     for g, (t, w) in enumerate(zip(ctx, heads(wuv_buf, i))))

    ctx = lax.fori_loop(0, 4, ctx_part, (jnp.zeros((16, D), F32),) * 4)
    issue_o(30, 38)
    ctx_ref[:B * H] = by_batch(ctx).astype(BF16).astype(F32)
    flat = jnp.concatenate([ctx_ref[pl.ds(h % H, B, stride=H), :] for h in range(H + 1)], axis=1)
    for j in reversed(range(8)):
        starts = [16 * _piece(j ^ FLIP_O[r], 8, SKEW_W + r * 32, 256) for r in range(8)]
        lhs_ref[j] = jnp.concatenate([flat[:, k:k + 64] for k in starts], axis=1)
    cols = [slice(i * 128, (i + 1) * 128) for i in range(4)]
    for b in range(B):
        for c in cols:
            mul_ref[b, c] = jnp.broadcast_to(lhs_ref[7, b:b + 1, c], (128, 128)).T

    w1 = w1_buf[...].reshape(M // 8, F // 128, 8, 128)
    hid = jnp.concatenate([_dot(xn, w1[:, i].reshape(M, 128)) for i in range(F // 128)], axis=1)
    hid = jax.nn.gelu(hid + b1_buf[...].astype(F32).reshape(1, F), approximate=True).astype(BF16)
    z = _dot(hid, w2_buf[...].reshape(F, M)) + b2_buf[...].astype(F32).reshape(1, M)
    gate = z * jax.nn.sigmoid(z)

    def project(j, s):
        pl.when(j == 0)(lambda: issue_o(38, 48))
        pl.when(j == 2)(lambda: issue_o(48, 56))
        pl.when(j == 4)(lambda: issue_o(56, 64))
        wait_filled(wo_buf.at[j], S_O + j)
        return s + _dot(lhs_ref[j].astype(BF16), wo_buf[j])

    base = x + lax.fori_loop(0, 7, project, jnp.zeros((B, M), F32)) * gate
    for e in ORDER_O[LAST_CUTS[GATED] // 16:]:
        for b in range(B):
            k = pl.ds(16 * e, 16)
            gmul_ref[b, k] = jnp.concatenate([mul_ref[b, k]] * 4, axis=1) * gate[b:b + 1]

    sub = _iota((8, 128), 0)
    part = [[None] * 4 for _ in range(B)]
    for n, (lo, hi) in enumerate(zip(LAST_CUTS, LAST_CUTS[1:])):
        if n == GATED:
            part = [[part[b][i] * gate[b:b + 1, c] + jnp.where(sub == 0, base[b:b + 1, c], 0.0)
                     for i, c in enumerate(cols)] for b in range(B)]
        wait_filled(wo_buf.at[7, lo:hi], S_LAST + n)
        for r in range(lo, hi, 8):
            w = wo_buf[7, r:r + 8].astype(F32)
            k = pl.ds(16 * ORDER_O[r // 16] + r % 16, 8)
            for b in range(B):
                for i, c in enumerate(cols):
                    t = w[:, c] * (gmul_ref[b, k, c] if n >= GATED else mul_ref[b, k])
                    part[b][i] = t if part[b][i] is None else part[b][i] + t

    def merge(lo, hi, k):
        m = (sub & k) != 0
        return jnp.where(m, hi, lo) + pltpu.roll(jnp.where(m, lo, hi), k, 0)

    r1 = [merge(part[0][i], part[1][i], 1) for i in range(4)]
    o_buf[...] = merge(merge(r1[0], r1[1], 2), merge(r1[2], r1[3], 2), 4).astype(BF16)
    o_copy = pltpu.make_async_copy(o_buf, o_hbm, sems.at[S_OUT])
    o_copy.start()
    o_copy.wait()


@jax.jit
def pallas_recurrent_scan__compressed_kv_cla__dense_activation_gelu__decode_kernel(
    A_x: jax.Array,
    A_c_kv: jax.Array,
    A_w_q: jax.Array,
    A_w_uk: jax.Array,
    A_w_uv: jax.Array,
    A_w_o: jax.Array,
    B_x: jax.Array,
    B_w1: jax.Array,
    B_b1: jax.Array,
    B_w2: jax.Array,
    B_b2: jax.Array,
):
    del B_x
    hbm = pl.BlockSpec(memory_space=pltpu.HBM)
    vmem = pltpu.VMEM
    w1_tiles = B_w1.reshape(M // 8, 8, F // 128, 128).transpose(0, 2, 1, 3).reshape(W1_VIEW)
    out = pl.pallas_call(
        _kernel,
        out_shape=jax.ShapeDtypeStruct((8, 128), BF16),
        in_specs=[hbm] * 10,
        out_specs=hbm,
        scratch_shapes=[
            vmem((C_ROUNDS, 128, 16, DC), BF16), vmem(W_VIEW, BF16), vmem(W_VIEW, BF16), vmem(W_VIEW, BF16),
            vmem((8, 512, M), BF16), vmem(W1_VIEW, BF16), vmem(W2_VIEW, BF16),
            vmem((4, B * H, 128), BF16), vmem((B * H, DC), F32), vmem((B * H, 128), F32), vmem((B * H, 128), F32),
            vmem((4, B * H, 1024), BF16), vmem((128, 1024), BF16),
            vmem((3 * H, D), F32), vmem((8, B, 512), F32), vmem((B, 512, 128), F32), vmem((B, 512, M), F32),
            vmem((8, 128), BF16), vmem((B, M), BF16), vmem((F,), BF16), vmem((M,), BF16),
            pltpu.SemaphoreType.DMA((S_LAST + len(LAST_CUTS) - 1,)),
        ],
        compiler_params=pltpu.CompilerParams(
            vmem_limit_bytes=100 * 1024 * 1024, disable_semaphore_checks=True, disable_bounds_checks=True),
    )(A_x.reshape(B, M), A_c_kv.reshape(C_VIEW), A_w_q.reshape(W_VIEW), A_w_uk.reshape(W_VIEW),
      A_w_uv.reshape(W_VIEW), A_w_o.reshape(O_VIEW), w1_tiles, B_b1, B_w2.reshape(W2_VIEW), B_b2)
    return out.reshape(M // 128, B, 128).transpose(1, 0, 2).reshape(B, 1, M)
```

```python
import jax
import jax.numpy as jnp
from jax import lax
import jax.experimental.pallas as pl
import jax.experimental.pallas.tpu as pltpu

F32 = jnp.float32
BF16 = jnp.bfloat16

B, H, SK, D, M, DC, F = 2, 32, 16384, 128, 512, 512, 1792
LOG2E = 1.4426950408889634
NN = (((1,), (0,)), ((), ()))
NT = (((1,), (1,)), ((), ()))

C_VIEW = (B * SK // 16, 16, DC)
W_VIEW = (M // 2, 2 * H, D)
O_VIEW = (H * D // 16, 16, M)
W1_VIEW = (F // 16, 64, 128)
W2_VIEW = (F // 16, 16, M)

ORDER_QK = (51, 27, 50, 26, 42, 34, 43, 35, 15, 18, 17, 55, 52, 57, 58, 12, 25, 49, 24, 48, 32, 40, 33, 41,
            19, 13, 14, 56, 59, 53, 54, 16, 46, 22, 23, 47, 7, 6, 30, 31, 38, 39, 63, 62, 8, 0, 20, 44, 45,
            21, 1, 9, 60, 61, 36, 37, 28, 29, 4, 5, 11, 2, 10, 3)
ORDER_VF = ((36, 37, 42, 4, 17, 12, 19, 13, 29, 28, 35, 34, 43, 5, 38, 39, 14, 16, 15, 18, 2, 41, 6, 11, 33,
             31, 32, 30, 7, 3, 10, 40, 20, 26, 22, 27, 45, 51, 50, 47, 8, 0, 9, 1, 52, 58, 59, 54, 24, 21,
             25, 23, 44, 49, 46, 48, 53, 56, 57, 55),
            (12, 17, 42, 16, 0, 29, 36, 28, 55, 54, 53, 43, 15, 18, 41, 52, 1, 37, 30, 6, 14, 19, 13, 40, 7,
             31, 2, 38, 27, 21, 26, 23, 11, 5, 32, 3, 44, 51, 59, 50, 39, 10, 4, 33, 20, 25, 22, 24, 58, 47,
             49, 45, 35, 8, 34, 9, 48, 57, 46, 56))
ORDER_C = (49, 17, 12, 44, 25, 36, 68, 57, 4, 65, 124, 41, 20, 9, 52, 60, 1, 33, 28, 6, 5, 24, 37, 56, 69,
           61, 0, 125, 64, 32, 29, 40, 8, 21, 53, 45, 13, 16, 48, 112, 80, 77, 109, 117, 72, 85, 104, 96,
           93, 92, 97, 101, 88, 89, 100, 113, 81, 76, 108, 84, 116, 73, 105, 7, 47, 15, 18, 50, 39, 26, 58,
           71, 42, 10, 23, 55, 127, 66, 34, 31, 63, 2, 27, 38, 19, 51, 14, 46, 59, 70, 3, 62, 126, 30, 35,
           67, 120, 54, 43, 11, 22, 102, 91, 123, 78, 83, 115, 110, 86, 75, 118, 107, 94, 99, 98, 95, 121,
           103, 90, 122, 87, 119, 106, 74, 114, 82, 111, 79)
ORDER_O = (30, 29, 31, 28, 5, 7, 4, 6, 15, 13, 14, 12, 25, 27, 24, 26, 2, 1, 3, 0, 8, 11, 9, 10, 18, 17,
           19, 16, 20, 23, 21, 22)
FLIP_O = (1, 1, 1, 0, 0, 5, 5, 4)
SKEW_C, SKEW_W, SKEW_W2 = 46, 14, 15
LAG = 26
HALVED = 12
LAST_CUTS = (0, 192, 320, 384, 432, 464, 480, 496, 512)
GATED = 3

C_ROUNDS = 16
S_Q, S_K, S_V, S_W1, S_W2, S_X, S_B1, S_B2, S_OUT, S_C = range(10)
S_O = S_C + C_ROUNDS
S_LAST = S_O + 7


def _loop(lo, hi, body):
    lax.fori_loop(lo, hi, lambda i, _: body(i), None)


def _dot(a, b, dims=NN):
    return lax.dot_general(a, b, dims, preferred_element_type=F32)


def _iota(shape, axis):
    return lax.broadcasted_iota(jnp.int32, shape, axis)


def _piece(j, rounds, first, n):
    first %= n
    i = first + 4 * j
    if first + 4 * (rounds - 1) < n:
        return i
    return i % n if isinstance(i, int) else jnp.where(i >= n, i - n, i)


def _kernel(x_hbm, ckv_hbm, wq_hbm, wuk_hbm, wuv_hbm, wo_hbm, w1_hbm, b1_hbm, w2_hbm, b2_hbm,
            o_hbm,
            c_buf, wq_buf, wuk_buf, wuv_buf, wo_buf, w1_buf, w2_buf,
            qa_ref, acc_ref, m_ref, l_ref, a_buf, e_buf, ctx_ref, lhs_ref, mul_ref, gmul_ref,
            o_buf, x_buf, b1_buf, b2_buf, sems):
    def round_qk(j):
        def one(r, t):
            hbm, buf, sem = (wq_hbm, wq_buf, S_Q) if r >= 8 else (wuk_hbm, wuk_buf, S_K)
            i = _piece(j, 8, SKEW_W + r % 8 * 32 + t, 256)
            return hbm.at[i], buf.at[i], sem
        return [lambda e=e: one(*divmod(e, 4)) for e in ORDER_QK]

    def round_vf(half, j):
        def one(r, t):
            if r < 8:
                i = _piece(j, 4, SKEW_W + r * 32 + half * 16 + t, 256)
                return wuv_hbm.at[i], wuv_buf.at[i], S_V
            second = half if r == 14 else r >= 11
            hbm, buf, sem, skew = (w2_hbm, w2_buf, S_W2, SKEW_W2) if second else (w1_hbm, w1_buf, S_W1, SKEW_W)
            i = _piece(j, 4, skew + (96 if r == 14 else (r - 8) % 3 * 32 + half * 16) + t, 112)
            return hbm.at[i], buf.at[i], sem
        return [lambda e=e: one(*divmod(e, 4)) for e in ORDER_VF[half]]

    def round_c(j):
        def one(r, t):
            i = r // 16 * 1024 + _piece(j, C_ROUNDS, SKEW_C + r % 16 * 64 + t, 1024)
            return ckv_hbm.at[i], c_buf.at[j, 4 * r + t], S_C + j
        return [lambda e=e: one(*divmod(e, 4)) for e in ORDER_C]

    def piece_o(n, lo=0, hi=16):
        j, e = n // 32, ORDER_O[n % 32]
        i = _piece(j ^ FLIP_O[e // 4], 8, SKEW_W + e // 4 * 32 + e % 4, 256)
        row = 16 * (e if j < 7 else n % 32)
        sem = S_O + j if j < 7 else S_LAST + sum(row >= c for c in LAST_CUTS[1:])
        return wo_hbm.at[i, lo:hi], wo_buf.at[j, row + lo:row + hi], sem

    stream_o = [lambda n=n: piece_o(n) for n in range(256 - HALVED)]
    halves_o = [lambda n=n, r=r: piece_o(n, r, r + 8) for n in range(256 - HALVED, 256) for r in (0, 8)]

    def start(piece, queue):
        src, dst, sem = piece()
        pltpu.make_async_copy(src, dst, sems.at[sem]).start(priority=queue)

    def queue1(pieces):
        return [p for n, p in enumerate(pieces) if n % 4 != 1]

    def issue(cur, nxt, lo=0, hi=64, end=()):
        ahead = (queue1(cur + nxt) + list(end))[LAG + 1:]
        for g in range(lo, min(hi, len(cur) // 4)):
            start(cur[4 * g + 1], 0)
            for p in ahead[3 * g:3 * g + 3]:
                start(p, 1)

    def issue_o(lo, hi):
        issue(stream_o, [], lo, hi, halves_o)

    def wait_filled(buf, sem):
        pltpu.make_async_copy(buf, buf, sems.at[sem]).wait()

    first = round_qk(0)
    start(first[0], 1)
    start(first[1], 0)
    for p in queue1(first)[1:LAG + 4]:
        start(p, 1)
    issue(first, round_qk(1), 1)
    for hbm, buf, sem in ((x_hbm, x_buf, S_X), (b1_hbm, b1_buf, S_B1), (b2_hbm, b2_buf, S_B2)):
        pltpu.make_async_copy(hbm, buf, sems.at[sem]).start()
    _loop(1, 4, lambda j: issue(round_qk(j), round_qk(j + 1)))

    pltpu.make_async_copy(x_hbm, x_buf, sems.at[S_X]).wait()
    x = x_buf[...].astype(F32)
    xc = x - jnp.mean(x, axis=-1, keepdims=True)
    var = jnp.mean(xc * xc, axis=-1, keepdims=True)
    xn = (xc * lax.rsqrt(var + 1e-5)).astype(BF16)

    e_buf[...] = (_iota((128, 1024), 1) // 8 == _iota((128, 1024), 0)).astype(F32).astype(BF16)

    def own_head(v):
        return jnp.where(_iota(v.shape, 0) % 8 == _iota(v.shape, 1) % 8, v, 0.0).astype(BF16)

    def heads(buf, i):
        w = buf[pl.ds(i * 64, 64)].reshape(128, 4, 8, D)
        return [w[:, g].reshape(1024, D) for g in range(4)]

    def by_batch(groups):
        return jnp.concatenate([t[8 * b:8 * b + 8] for b in range(B) for t in groups], axis=0)

    xf = xn.astype(F32)
    x16 = jnp.concatenate([jnp.broadcast_to(xf[b:b + 1], (8, M)) for b in range(B)], axis=0).astype(BF16)
    for i in range(4):
        a_buf[i, :16] = own_head(_dot(x16[:, i * 128:(i + 1) * 128], e_buf[...]))
    m_ref[...] = jnp.full((B * H, 128), -jnp.inf, F32)
    l_ref[...] = jnp.zeros((B * H, 128), F32)
    acc_ref[...] = jnp.zeros((B * H, DC), F32)
    _loop(4, 7, lambda j: issue(round_qk(j), round_qk(j + 1)))
    issue(round_qk(7), round_vf(0, 0))
    issue(round_vf(0, 0), round_vf(0, 1))
    issue(round_vf(0, 1), round_vf(0, 2), 0, 8)

    wait_filled(wq_buf, S_Q)
    wait_filled(wuk_buf, S_K)

    def q_part(i, q):
        pl.when(i == 2)(lambda: issue(round_vf(0, 1), round_vf(0, 2), 8))
        return tuple(t + _dot(a_buf[i, :16], w) for t, w in zip(q, heads(wq_buf, i)))

    q = [t.astype(BF16) for t in lax.fori_loop(0, 4, q_part, (jnp.zeros((16, D), F32),) * 4)]

    def qa_part(i):
        pl.when(i == 0)(lambda: issue(round_vf(0, 2), round_vf(0, 3)))
        pl.when(i == 1)(lambda: issue(round_vf(0, 3), round_c(0)))
        pl.when(i == 2)(lambda: issue(round_c(0), round_c(1), 0, 16))
        pl.when(i == 3)(lambda: issue(round_c(0), round_c(1), 16))
        r = by_batch([_dot(t, w, NT) for t, w in zip(q, heads(wuk_buf, i))])
        qa_ref[i] = _dot(own_head(r * (D ** -0.5 * LOG2E)), e_buf[...], NT).astype(BF16)

    _loop(0, 4, qa_part)
    issue(round_c(1), round_c(2), 0, 16)

    def feed(j, k):
        last = C_ROUNDS - 1
        pl.when(j < last)(lambda: issue(round_c(j), round_c(j + 1), 8 * k, 8 * k + 8))
        pl.when(j == last)(lambda: issue(round_c(last), round_vf(1, 0), 8 * k, 8 * k + 8))
        n = (j - C_ROUNDS) * 2 + k // 2
        pl.when(j > last)(lambda: issue(round_vf(1, n), round_vf(1, n + 1), k % 2 * 8, k % 2 * 8 + 8))

    def block(j):
        for b in range(B):
            feed(j + 1 + b, 2 - 2 * b)
            if b == 0:
                wait_filled(c_buf.at[j], S_C + j)
            rows = pl.ds(b * H, H)
            keys = (j, pl.ds(b * 64, 64))
            qa = jnp.concatenate([qa_ref[i, rows] for i in range(4)], axis=1)
            sc = _dot(qa, c_buf[keys].reshape(1024, DC), NT)
            m_prev = m_ref[rows, :]
            m_new = jnp.maximum(m_prev, jnp.max(sc, axis=1, keepdims=True))
            p = [jnp.exp2(sc[:, i * 128:(i + 1) * 128] - m_new) for i in range(8)]
            alpha = jnp.exp2(m_prev - m_new)
            l_ref[rows, :] = alpha * l_ref[rows, :] + sum(p)
            m_ref[rows, :] = m_new
            p = jnp.concatenate(p, axis=1).astype(BF16)
            feed(j + 1 + b, 3 - 2 * b)
            pv = _dot(p, c_buf[keys].reshape(1024, DC))
            acc_ref[rows, :] = acc_ref[rows, :] * jnp.concatenate([alpha] * 4, axis=1) + pv

    _loop(0, C_ROUNDS, block)

    pc = acc_ref[...] / jnp.sum(l_ref[...], axis=1, keepdims=True)
    pc = jnp.concatenate([pc[b * H + 8 * g:b * H + 8 * g + 8, i * 128:(i + 1) * 128]
                          for i in range(4) for g in range(4) for b in range(B)], axis=0)
    a_buf[...] = own_head(_dot(pc.astype(BF16), e_buf[...])).reshape(4, B * H, 1024)
    issue(round_vf(1, 3), stream_o)
    issue_o(0, 22)
    wait_filled(wuv_buf, S_V)
    wait_filled(w1_buf, S_W1)
    wait_filled(w2_buf, S_W2)
    pltpu.make_async_copy(b1_hbm, b1_buf, sems.at[S_B1]).wait()
    pltpu.make_async_copy(b2_hbm, b2_buf, sems.at[S_B2]).wait()

    def ctx_part(i, ctx):
        pl.when(i == 2)(lambda: issue_o(22, 30))
        return tuple(t + _dot(a_buf[i, 16 * g:16 * g + 16], w)
                     for g, (t, w) in enumerate(zip(ctx, heads(wuv_buf, i))))

    ctx = lax.fori_loop(0, 4, ctx_part, (jnp.zeros((16, D), F32),) * 4)
    issue_o(30, 38)
    ctx_ref[:B * H] = by_batch(ctx).astype(BF16).astype(F32)
    flat = jnp.concatenate([ctx_ref[pl.ds(h % H, B, stride=H), :] for h in range(H + 1)], axis=1)
    for j in reversed(range(8)):
        starts = [16 * _piece(j ^ FLIP_O[r], 8, SKEW_W + r * 32, 256) for r in range(8)]
        lhs_ref[j] = jnp.concatenate([flat[:, k:k + 64] for k in starts], axis=1)
    cols = [slice(i * 128, (i + 1) * 128) for i in range(4)]
    for b in range(B):
        for c in cols:
            mul_ref[b, c] = jnp.broadcast_to(lhs_ref[7, b:b + 1, c], (128, 128)).T

    w1 = w1_buf[...].reshape(M // 8, F // 128, 8, 128)
    hid = jnp.concatenate([_dot(xn, w1[:, i].reshape(M, 128)) for i in range(F // 128)], axis=1)
    hid = jax.nn.gelu(hid + b1_buf[...].astype(F32).reshape(1, F), approximate=True).astype(BF16)
    z = _dot(hid, w2_buf[...].reshape(F, M)) + b2_buf[...].astype(F32).reshape(1, M)
    gate = z * jax.nn.sigmoid(z)

    def project(j, s):
        pl.when(j == 0)(lambda: issue_o(38, 48))
        pl.when(j == 2)(lambda: issue_o(48, 56))
        pl.when(j == 4)(lambda: issue_o(56, 64))
        wait_filled(wo_buf.at[j], S_O + j)
        return s + _dot(lhs_ref[j].astype(BF16), wo_buf[j])

    base = x + lax.fori_loop(0, 7, project, jnp.zeros((B, M), F32)) * gate
    for e in ORDER_O[LAST_CUTS[GATED] // 16:]:
        for b in range(B):
            k = pl.ds(16 * e, 16)
            gmul_ref[b, k] = jnp.concatenate([mul_ref[b, k]] * 4, axis=1) * gate[b:b + 1]

    sub = _iota((8, 128), 0)
    part = [[None] * 4 for _ in range(B)]
    for n, (lo, hi) in enumerate(zip(LAST_CUTS, LAST_CUTS[1:])):
        if n == GATED:
            part = [[part[b][i] * gate[b:b + 1, c] + jnp.where(sub == 0, base[b:b + 1, c], 0.0)
                     for i, c in enumerate(cols)] for b in range(B)]
        wait_filled(wo_buf.at[7, lo:hi], S_LAST + n)
        for r in range(lo, hi, 8):
            w = wo_buf[7, r:r + 8].astype(F32)
            k = pl.ds(16 * ORDER_O[r // 16] + r % 16, 8)
            for b in range(B):
                for i, c in enumerate(cols):
                    t = w[:, c] * (gmul_ref[b, k, c] if n >= GATED else mul_ref[b, k])
                    part[b][i] = t if part[b][i] is None else part[b][i] + t

    def merge(lo, hi, k):
        m = (sub & k) != 0
        return jnp.where(m, hi, lo) + pltpu.roll(jnp.where(m, lo, hi), k, 0)

    r1 = [merge(part[0][i], part[1][i], 1) for i in range(4)]
    o_buf[...] = merge(merge(r1[0], r1[1], 2), merge(r1[2], r1[3], 2), 4).astype(BF16)
    o_copy = pltpu.make_async_copy(o_buf, o_hbm, sems.at[S_OUT])
    o_copy.start()
    o_copy.wait()


@jax.jit
def pallas_recurrent_scan__compressed_kv_cla__dense_activation_gelu__decode_kernel(
    A_x: jax.Array,
    A_c_kv: jax.Array,
    A_w_q: jax.Array,
    A_w_uk: jax.Array,
    A_w_uv: jax.Array,
    A_w_o: jax.Array,
    B_x: jax.Array,
    B_w1: jax.Array,
    B_b1: jax.Array,
    B_w2: jax.Array,
    B_b2: jax.Array,
):
    del B_x
    hbm = pl.BlockSpec(memory_space=pltpu.HBM)
    vmem = pltpu.VMEM
    w1_tiles = B_w1.reshape(M // 8, 8, F // 128, 128).transpose(0, 2, 1, 3).reshape(W1_VIEW)
    out = pl.pallas_call(
        _kernel,
        out_shape=jax.ShapeDtypeStruct((8, 128), BF16),
        in_specs=[hbm] * 10,
        out_specs=hbm,
        scratch_shapes=[
            vmem((C_ROUNDS, 128, 16, DC), BF16), vmem(W_VIEW, BF16), vmem(W_VIEW, BF16), vmem(W_VIEW, BF16),
            vmem((8, 512, M), BF16), vmem(W1_VIEW, BF16), vmem(W2_VIEW, BF16),
            vmem((4, B * H, 128), BF16), vmem((B * H, DC), F32), vmem((B * H, 128), F32), vmem((B * H, 128), F32),
            vmem((4, B * H, 1024), BF16), vmem((128, 1024), BF16),
            vmem((3 * H, D), F32), vmem((8, B, 512), F32), vmem((B, 512, 128), F32), vmem((B, 512, M), F32),
            vmem((8, 128), BF16), vmem((B, M), BF16), vmem((F,), BF16), vmem((M,), BF16),
            pltpu.SemaphoreType.DMA((S_LAST + len(LAST_CUTS) - 1,)),
        ],
        compiler_params=pltpu.CompilerParams(
            vmem_limit_bytes=100 * 1024 * 1024, disable_semaphore_checks=True, disable_bounds_checks=True),
    )(A_x.reshape(B, M), A_c_kv.reshape(C_VIEW), A_w_q.reshape(W_VIEW), A_w_uk.reshape(W_VIEW),
      A_w_uv.reshape(W_VIEW), A_w_o.reshape(O_VIEW), w1_tiles, B_b1, B_w2.reshape(W2_VIEW), B_b2)
    return out.reshape(M // 128, B, 128).transpose(1, 0, 2).reshape(B, 1, M)
```
